```python
import os as _os
_os.environ.setdefault("JAX_PLATFORMS", "cpu")
import jax
import jax.numpy as jnp

def _softmax(x, axis=-1):
    return jax.nn.softmax(x, axis=axis)
def _gelu(x):
    return jax.nn.gelu(x, approximate=True)
def _silu(x):
    return jax.nn.silu(x)
def _sigmoid(x):
    return jax.nn.sigmoid(x)
def _layernorm(x, axis=-1, eps=1e-5):
    m = jnp.mean(x, axis=axis, keepdims=True)
    v = jnp.var(x, axis=axis, keepdims=True)
    return (x - m) / jnp.sqrt(v + eps)
def _scatter_add(tgt, idx, src, axis=0):
    return tgt.at[idx].add(src)
def _segment_sum(src, seg, n):
    return jax.ops.segment_sum(src, seg, n)
class _Rng:
    def __init__(self, key):
        self._k = key
    def _next(self):
        self._k, sub = jax.random.split(self._k)
        return sub
    def normal(self, shape):
        return jax.random.normal(self._next(), shape, dtype=jnp.bfloat16)
    def randint(self, lo, hi, shape):
        return jax.random.randint(self._next(), shape, lo, hi, dtype=jnp.int32)
    def uniform(self, shape, lo=0.0, hi=1.0):
        return jax.random.uniform(self._next(), shape, jnp.bfloat16, lo, hi)
    def permutation(self, n):
        return jax.random.permutation(self._next(), n)


kernel_name = 'sequential_preLN__softmax_full_mha__dense_activation_gelu__prompt'

def setup_inputs():
    _rng = _Rng(jax.random.key(int.from_bytes(__import__("os").urandom(4), "little")))
    _w = (lambda a: (lambda t: t.astype(jnp.bfloat16) if jnp.issubdtype(t.dtype, jnp.floating) else t)(jnp.asarray(a)))
    def _A_setup():
        B, S, D = 1, 2048, 640
        return {
            "x": _w((lambda *s: _rng.normal(s) * 0.05)(B, S, D)),
            "wqkv": _w((lambda *s: _rng.normal(s) * 0.05)(D, 3 * D)),
            "wo": _w((lambda *s: _rng.normal(s) * 0.05)(D, D)),
        }
    _A_in = _A_setup()

    def _B_setup():
        B, S, D, F = 1, 2048, 640, 1536
        return {
            "x": _w((lambda *s: _rng.normal(s) * 0.05)(B, S, D)),
            "w1": _w((lambda *s: _rng.normal(s) * 0.4)(D, F) * (D ** -0.5)),
            "b1": _w((lambda *s: _rng.normal(s) * 0.4)(F) * 0.01),
            "w2": _w((lambda *s: _rng.normal(s) * 0.4)(F, D) * (F ** -0.5)),
            "b2": _w((lambda *s: _rng.normal(s) * 0.05)(D) * 0.01),
        }
    _B_in = _B_setup()

    return {
        "A_x": _A_in["x"],
        "A_wqkv": _A_in["wqkv"],
        "A_wo": _A_in["wo"],
        "B_x": _B_in["x"],
        "B_w1": _B_in["w1"],
        "B_b1": _B_in["b1"],
        "B_w2": _B_in["w2"],
        "B_b2": _B_in["b2"],
    }

def reference(A_x, A_wqkv, A_wo, B_x, B_w1, B_b1, B_w2, B_b2):
    def _A_ref(x, wqkv, wo):
        B, S, D = x.shape
        H = 32; Dh = D // H
        qkv = (lambda x, *d: x.transpose(*d))((x @ wqkv).reshape(B, S, 3, H, Dh), 2, 0, 3, 1, 4)
        q, k, v = qkv[0], qkv[1], qkv[2]
        scale = Dh ** -0.5
        scores = jnp.einsum("bhqd,bhkd->bhqk", q, k) * scale
        p = _softmax(scores, axis=-1)
        o = jnp.einsum("bhqk,bhkd->bhqd", p, v)
        return (lambda x, *d: x.transpose(*d))(o, 0, 2, 1, 3).reshape(B, S, D) @ wo

    def _B_ref(x, w1, b1, w2, b2):
        h = jnp.einsum("bsd,df->bsf", x, w1) + b1
        h = _gelu(h)
        return jnp.einsum("bsf,fd->bsd", h, w2) + b2

    x = A_x
    h = x + _A_ref(_layernorm(x, axis=-1), A_wqkv, A_wo)
    h2 = h + _B_ref(_layernorm(h, axis=-1), B_w1, B_b1, B_w2, B_b2)
    return h2
```

```python
import functools
import math

import jax
import jax.numpy as jnp
from jax import lax
import jax.experimental.pallas as pl
import jax.experimental.pallas.tpu as pltpu

S = 2048
D = 640
H = 32
DH = 20
F = 1536
EPS = 1e-5
NG = 5
NGT = 9
LOG2E = 1.4426950408889634

F32 = jnp.float32
BF16 = jnp.bfloat16


def _ln(x):
    m = jnp.mean(x, axis=-1, keepdims=True)
    xc = x - m
    v = jnp.mean(xc * xc, axis=-1, keepdims=True)
    return xc * lax.rsqrt(v + EPS)


def _gelu(x):
    c = math.sqrt(2.0 / math.pi)
    inner = x * (c + (c * 0.044715) * (x * x))
    return x * (0.5 + 0.5 * jnp.tanh(inner))


def make_kernel(TQ, CK, RC):
    NQ = S // TQ
    NCK = S // CK
    NRC = S // RC

    def kernel(x_ref, wqkv_ref, wo_ref, w1_ref, b1_ref, w2_ref, b2_ref, o_ref,
               wt_ref, kg_ref, qtg_ref, vt_ref, s0_ref, s1_ref, m0_ref, m1_ref,
               qm_ref, ot_ref):
        i = pl.program_id(0)

        def head_group(h):
            start = h * DH
            g0 = start // 128
            g1 = (start + DH - 1) // 128
            g = jnp.where(g0 != g1, NG + g0, g0)
            return g, start

        def prep_q(h, qb, slot):
            g, start = head_group(h)
            row = lax.broadcasted_iota(jnp.int32, (128, TQ), 0)
            keep = ((row - start) & 127) < DH
            qt = qtg_ref[g, qb].astype(F32)
            qm_ref[slot] = jnp.where(keep, qt, 0.0).astype(BF16)
            return g

        def stage_a_chunk(g, slot, s_ref, c, m8):
            s = jnp.dot(kg_ref[g, pl.ds(c * CK, CK), :], qm_ref[slot],
                        preferred_element_type=F32)
            s_ref[pl.ds(c * CK, CK), :] = s
            pm = jnp.max(s.reshape(CK // 8, 8, TQ), axis=0)
            return pm if m8 is None else jnp.maximum(m8, pm)

        def finish_m(m8, m_ref):
            m = jnp.max(m8, axis=0, keepdims=True)
            m_ref[...] = jnp.broadcast_to(m, (8, TQ))

        def stage_b_chunk(h, s_ref, m, c, acc):
            s = s_ref[pl.ds(c * CK, CK), :].reshape(CK // 8, 8, TQ)
            p = jnp.exp2(s - m[None]).reshape(CK, TQ).astype(BF16)
            o = jnp.dot(vt_ref[h, :, pl.ds(c * CK, CK)], p,
                        preferred_element_type=F32)
            return o if acc is None else acc + o

        @pl.when(i == 0)
        def _prologue():
            for b in range(NG):
                wt_ref[pl.ds(b * 128, 128), :] = (
                    wqkv_ref[:, pl.ds(b * 128, 128)].astype(F32).T.astype(BF16))
                wt_ref[pl.ds(D + b * 128, 128), :] = (
                    wqkv_ref[:, pl.ds(2 * D + b * 128, 128)].astype(F32).T.astype(BF16))

            qscale = (DH ** -0.5) * LOG2E
            lane = lax.broadcasted_iota(jnp.int32, (RC, 128), 1)
            r24 = lax.broadcasted_iota(jnp.int32, (24, RC), 0)
            r8 = lax.broadcasted_iota(jnp.int32, (8, RC), 0)
            tail = jnp.where(r8 == 0, 1.0, 0.0).astype(F32)

            def chunk(r, carry):
                r0 = pl.multiple_of(r * RC, RC)
                xn = _ln(x_ref[pl.ds(r0, RC), :].astype(F32)).astype(BF16)
                k = jnp.dot(xn, wqkv_ref[:, pl.ds(D, D)], preferred_element_type=F32)
                for g in range(NG):
                    kg_ref[g, pl.ds(r0, RC), :] = k[:, g * 128:(g + 1) * 128].astype(BF16)
                for b in range(NG - 1):
                    kg_ref[NG + b, pl.ds(r0, RC), :] = jnp.where(
                        lane >= 64, k[:, b * 128:(b + 1) * 128],
                        k[:, (b + 1) * 128:(b + 2) * 128]).astype(BF16)
                qv = lax.dot_general(wt_ref[...], xn, (((1,), (1,)), ((), ())),
                                     preferred_element_type=F32)
                qt = (qv[:D] * qscale).astype(BF16)
                qb = r // (TQ // RC)
                c0 = pl.multiple_of((r % (TQ // RC)) * RC, RC)
                for g in range(NG):
                    qtg_ref[g, qb, :, pl.ds(c0, RC)] = qt[g * 128:(g + 1) * 128]
                for b in range(NG - 1):
                    qtg_ref[NG + b, qb, pl.ds(0, 64), pl.ds(c0, RC)] = (
                        qt[(b + 1) * 128:(b + 1) * 128 + 64])
                    qtg_ref[NG + b, qb, pl.ds(64, 64), pl.ds(c0, RC)] = (
                        qt[b * 128 + 64:(b + 1) * 128])
                for j in range(H // 2):
                    ve = qv[D + 40 * j:D + 40 * j + 24]
                    ve = jnp.where(r24 < DH, ve, 0.0)
                    vt_ref[2 * j, :, pl.ds(r0, RC)] = jnp.concatenate(
                        [ve, tail], axis=0).astype(BF16)
                    vo = qv[D + 40 * j + 16:D + 40 * j + 40]
                    vo = jnp.where(r24 >= 4, vo, 0.0)
                    vt_ref[2 * j + 1, :, pl.ds(r0, RC)] = jnp.concatenate(
                        [vo, tail], axis=0).astype(BF16)
                return carry

            lax.fori_loop(0, NRC, chunk, 0)

            g = prep_q(0, 0, 0)
            m8 = None
            for c in range(NCK):
                m8 = stage_a_chunk(g, 0, s0_ref, c, m8)
            finish_m(m8, m0_ref)

        r8q = lax.broadcasted_iota(jnp.int32, (8, TQ), 0)

        def pair(j, carry):
            h0 = 2 * j
            g = prep_q(h0 + 1, i, 1)
            m = m0_ref[...]
            m8 = None
            acc = None
            for c in range(NCK):
                m8 = stage_a_chunk(g, 1, s1_ref, c, m8)
                acc = stage_b_chunk(h0, s0_ref, m, c, acc)
            finish_m(m8, m1_ref)
            oe = acc[:24] * (1.0 / acc[24:25])
            hn = (h0 + 2) % H
            qn = jnp.minimum(i + (h0 + 2) // H, NQ - 1)
            g = prep_q(hn, qn, 0)
            m = m1_ref[...]
            m8 = None
            acc = None
            for c in range(NCK):
                m8 = stage_a_chunk(g, 0, s0_ref, c, m8)
                acc = stage_b_chunk(h0 + 1, s1_ref, m, c, acc)
            finish_m(m8, m0_ref)
            oo = acc[:24] * (1.0 / acc[24:25])
            base = pl.multiple_of(j * 40, 8)
            ot_ref[pl.ds(base, 16), :] = oe[:16]
            ot_ref[pl.ds(base + 16, 8), :] = jnp.where(r8q < 4, oe[16:24], oo[:8])
            ot_ref[pl.ds(base + 24, 16), :] = oo[8:24]
            return carry

        lax.fori_loop(0, H // 2, pair, 0)

        o = ot_ref[...].T.astype(BF16)
        r0 = pl.multiple_of(i * TQ, TQ)
        h = x_ref[pl.ds(r0, TQ), :].astype(F32) + jnp.dot(
            o, wo_ref[...], preferred_element_type=F32)
        hn = _ln(h).astype(BF16)
        a = jnp.dot(hn, w1_ref[...], preferred_element_type=F32) + b1_ref[...].astype(F32)
        a = _gelu(a).astype(BF16)
        y = jnp.dot(a, w2_ref[...], preferred_element_type=F32) + b2_ref[...].astype(F32)
        o_ref[...] = (h + y).astype(o_ref.dtype)

    return kernel


def build(TQ=512, CK=256, RC=256):
    NQ = S // TQ

    @jax.jit
    def fn(A_x, A_wqkv, A_wo, B_x, B_w1, B_b1, B_w2, B_b2):
        x = A_x.reshape(S, D)
        full = lambda shape: pl.BlockSpec(shape, lambda i: (0,) * len(shape))
        out = pl.pallas_call(
            make_kernel(TQ, CK, RC),
            grid=(NQ,),
            in_specs=[full((S, D)), full((D, 3 * D)), full((D, D)), full((D, F)),
                      full((1, F)), full((F, D)), full((1, D))],
            out_specs=pl.BlockSpec((TQ, D), lambda i: (i, 0)),
            out_shape=jax.ShapeDtypeStruct((S, D), BF16),
            scratch_shapes=[
                pltpu.VMEM((2 * D, D), BF16),
                pltpu.VMEM((NGT, S, 128), BF16),
                pltpu.VMEM((NGT, NQ, 128, TQ), BF16),
                pltpu.VMEM((H, 32, S), BF16),
                pltpu.VMEM((S, TQ), F32),
                pltpu.VMEM((S, TQ), F32),
                pltpu.VMEM((8, TQ), F32),
                pltpu.VMEM((8, TQ), F32),
                pltpu.VMEM((2, 128, TQ), BF16),
                pltpu.VMEM((D, TQ), F32),
            ],
            compiler_params=pltpu.CompilerParams(
                dimension_semantics=("arbitrary",),
                vmem_limit_bytes=100 * 1024 * 1024),
        )(x, A_wqkv, A_wo, B_w1, B_b1.reshape(1, F), B_w2, B_b2.reshape(1, D))
        return out.reshape(1, S, D)

    return fn


_FN = build()


@jax.jit
def pallas_sequential_preLN__softmax_full_mha__dense_activation_gelu__prompt_kernel(
    A_x: jax.Array,
    A_wqkv: jax.Array,
    A_wo: jax.Array,
    B_x: jax.Array,
    B_w1: jax.Array,
    B_b1: jax.Array,
    B_w2: jax.Array,
    B_b2: jax.Array,
):
    return _FN(A_x, A_wqkv, A_wo, B_x, B_w1, B_b1, B_w2, B_b2)
```

```python
import math

import jax
import jax.numpy as jnp
from jax import lax
import jax.experimental.pallas as pl
import jax.experimental.pallas.tpu as pltpu

S = 2048
D = 640
H = 32
DH = 20
F = 1536
EPS = 1e-5
NG = D // 128
NPAIR = H // 2
LOG2E = 1.4426950408889634

F32 = jnp.float32
BF16 = jnp.bfloat16
U32 = jnp.uint32

TQ = 512
CK = 128
NQ = S // TQ
NCK = S // CK
NT = TQ // 128


def _ln(x):
    m = jnp.mean(x, axis=-1, keepdims=True)
    xc = x - m
    v = jnp.mean(xc * xc, axis=-1, keepdims=True)
    return xc * lax.rsqrt(v + EPS)


def _gelu(x):
    c = math.sqrt(2.0 / math.pi)
    inner = x * (c + (c * 0.044715) * (x * x))
    return x * (0.5 + 0.5 * jnp.tanh(inner))


class _NoScope:
    def __enter__(self):
        return self

    def __exit__(self, *a):
        return False


def _make_kernel(NH, ESPLIT, OFF, XCH, PROF):
    NGRP = H // NH
    NOFF = len(OFF)
    NV = 16 * NOFF
    HPI = H // NQ
    scope = jax.named_scope if PROF else (lambda name: _NoScope())

    def kernel(x_hbm, wqkv_hbm, wo_hbm, w1_hbm, b1_ref, w2_hbm, b2_ref, o_ref,
               x_ref, wk_ref, wqv_ref, wo_ref, w1_ref, w2_ref,
               xn_ref, wt_ref, kp_ref, qh_ref, vt_ref, s_ref, m_ref, ot_ref,
               kw_ref, kb_ref, qth_ref, qb_ref, zero_ref, xsem, wsem):
        i = pl.program_id(0)

        def x_copy(r):
            a, b = XCH[r]
            return pltpu.make_async_copy(
                x_hbm.at[pl.ds(a, b - a), :], x_ref.at[pl.ds(a, b - a), :],
                xsem.at[r])

        wk_copy = pltpu.make_async_copy(wqkv_hbm.at[:, pl.ds(D, D)], wk_ref, wsem.at[0])
        wq_copy = pltpu.make_async_copy(wqkv_hbm.at[:, pl.ds(0, D)], wqv_ref.at[0], wsem.at[1])
        wv_copy = pltpu.make_async_copy(wqkv_hbm.at[:, pl.ds(2 * D, D)], wqv_ref.at[1], wsem.at[2])
        wo_copy = pltpu.make_async_copy(wo_hbm, wo_ref, wsem.at[3])
        w1_copy = pltpu.make_async_copy(w1_hbm, w1_ref, wsem.at[4])
        w2_copy = pltpu.make_async_copy(w2_hbm, w2_ref, wsem.at[5])

        def split_n(n):
            if isinstance(n, int):
                return n % H, min(n // H, NQ - 1)
            return n % H, jnp.minimum(n // H, NQ - 1)

        def prep_qb(n, u):
            h, qb = split_n(n)
            e = u % 2
            for a in range(2 * e, 2 * e + 3):
                q8 = qth_ref[h // 2, qb, pl.ds(8 * a, 8), :]
                for r in range(8):
                    d = 8 * a + r - DH * e
                    if 0 <= d < DH:
                        qb_ref[u, d] = jnp.broadcast_to(q8[r:r + 1], (8, TQ))

        def scores_mxu(n, u, r0, nr, m8):
            h, qb = split_n(n)
            e = u % 2
            kd = 48 if e else 32
            k = pltpu.bitcast(kp_ref[h // 2, pl.ds(r0 // 2, nr // 2), :], BF16)
            q = pltpu.bitcast(qh_ref[h // 2, qb, pl.ds(16 * e, kd // 2), :], BF16)
            s = jnp.dot(k[:, :kd], q, preferred_element_type=F32)
            s_ref[u, pl.ds(r0, nr), :] = s
            pm = jnp.max(s.reshape(nr // 8, 8, TQ), axis=0)
            return pm if m8 is None else jnp.maximum(m8, pm)

        def scores_vpu(n, u, p, m8):
            h, _ = split_n(n)
            acc = [None] * NT
            for jd in range(DH // 2):
                lo = kb_ref[h, jd, pl.ds(p * 8, 8), :]
                hi = kb_ref[h, jd + DH // 2, pl.ds(p * 8, 8), :]
                for t in range(NT):
                    a = lo * qb_ref[u, jd, :, pl.ds(t * 128, 128)]
                    acc[t] = a if acc[t] is None else acc[t] + a
                    acc[t] = acc[t] + hi * qb_ref[u, jd + DH // 2, :, pl.ds(t * 128, 128)]
            row = OFF[p // 2] * CK + (p % 2) * 8
            for t in range(NT):
                s_ref[u, pl.ds(row, 8), pl.ds(t * 128, 128)] = acc[t]
            return jnp.maximum(m8, jnp.concatenate(acc, axis=1))

        def finish_m(m8, u):
            m = jnp.max(m8, axis=0, keepdims=True)
            m_ref[u] = jnp.broadcast_to(m, (8, TQ))

        def softmax_pv(h, u, m, c, acc):
            s = s_ref[u, pl.ds(c * CK, CK), :].reshape(CK // 8, 8, TQ)
            p = jnp.exp2(s - m[None]).reshape(CK, TQ)
            o = jnp.dot(vt_ref[h, :, pl.ds(c * CK, CK)], p,
                        preferred_element_type=F32)
            if acc is None:
                return (zero_ref[...] + o) if u > 0 else o
            return acc + o

        def ln_rows(a, b):
            for r0 in range(a, b, 256):
                xn_ref[pl.ds(r0, 256), :] = _ln(
                    x_ref[pl.ds(r0, 256), :].astype(F32)).astype(BF16)

        def kproj_rows(a, b):
            lane = lax.broadcasted_iota(jnp.int32, (128, 128), 1)
            for r0 in range(a, b, 256):
                k = jnp.dot(xn_ref[pl.ds(r0, 256), :], wk_ref[...],
                            preferred_element_type=F32)
                ku = pltpu.bitcast(k.astype(BF16), U32)
                for j in range(NPAIR):
                    start = 2 * DH * j
                    g0, g1 = start // 128, (start + 2 * DH - 1) // 128
                    kk = ku[:, g0 * 128:(g0 + 1) * 128]
                    if g1 != g0:
                        kk = jnp.where(lane >= 64, kk, ku[:, g1 * 128:(g1 + 1) * 128])
                    sh = (128 - start % 128) % 128
                    if sh:
                        kk = pltpu.roll(kk, sh, 1)
                    kp_ref[j, pl.ds(r0 // 2, 128), :] = kk

        def build_kw():
            for j in range(NPAIR):
                ku = jnp.concatenate(
                    [kp_ref[j, pl.ds(c * CK // 2, 8), :] for c in OFF], axis=0)
                kk = pltpu.bitcast(ku, BF16).astype(F32)
                kb = pltpu.bitcast(kk, U32)
                kw_ref[j] = ((pltpu.roll(kb, 128 - DH // 2, 1) & jnp.uint32(0xFFFF0000))
                             | (kb >> 16))

        @pl.when(i == 0)
        def _prologue():
            with scope("p_k"):
                x_copy(0).start()
                wk_copy.start()
                zero_ref[...] = jnp.zeros((24, TQ), F32)
                x_copy(1).start()
                x_copy(0).wait()
                x_copy(2).start()
                ln_rows(*XCH[0])
                wk_copy.wait()
                x_copy(1).wait()
                x_copy(3).start()
                ln_rows(*XCH[1])
                kproj_rows(*XCH[0])
                x_copy(2).wait()
                wq_copy.start()
                wv_copy.start()
                ln_rows(*XCH[2])
                kproj_rows(*XCH[1])
                x_copy(3).wait()
                ln_rows(*XCH[3])
                kproj_rows(*XCH[2])
                wq_copy.wait()
                wv_copy.wait()
                wo_copy.start()
                w1_copy.start()
                w2_copy.start()
                kproj_rows(*XCH[3])
                build_kw()
                for t in range(2):
                    for b in range(NG):
                        wt_ref[pl.ds(t * D + b * 128, 128), :] = (
                            wqv_ref[t, :, pl.ds(b * 128, 128)].astype(F32).T.astype(BF16))

            qscale = (DH ** -0.5) * LOG2E
            r24 = lax.broadcasted_iota(jnp.int32, (24, TQ), 0)
            r32 = lax.broadcasted_iota(jnp.int32, (32, TQ), 0)

            def qv_step(r, carry):
                r0 = pl.multiple_of(r * TQ, TQ)
                for hh in range(HPI):
                    kw = kw_ref[r * (HPI // 2) + hh // 2]
                    for jd in range(DH // 2):
                        l = DH * (hh % 2) + jd
                        w = jnp.broadcast_to(kw[:, l:l + 1], (NV, 128))
                        kb_ref[r * HPI + hh, jd] = pltpu.bitcast(w << 16, F32)
                        kb_ref[r * HPI + hh, jd + DH // 2] = pltpu.bitcast(
                            w & jnp.uint32(0xFFFF0000), F32)
                qv = lax.dot_general(wt_ref[...], xn_ref[pl.ds(r0, TQ), :],
                                     (((1,), (1,)), ((), ())),
                                     preferred_element_type=F32)
                zero16 = jnp.zeros((8, TQ), U32)
                for j in range(NPAIR):
                    q = qv[40 * j:40 * j + 48] * qscale
                    qe = jnp.where(r32 < DH, q[:32], 0.0).astype(BF16)
                    qo = jnp.where((r32 >= 4) & (r32 < 24), q[16:48], 0.0).astype(BF16)
                    qh_ref[j, r, pl.ds(0, 16), :] = pltpu.bitcast(qe, U32)
                    qh_ref[j, r, pl.ds(16, 8), :] = zero16
                    qh_ref[j, r, pl.ds(24, 16), :] = pltpu.bitcast(qo, U32)
                    qth_ref[j, r] = q[:40].astype(BF16).astype(F32)
                for j in range(NPAIR):
                    ve = qv[D + 40 * j:D + 40 * j + 24]
                    ve = jnp.where(r24 < DH, ve, jnp.where(r24 == DH, 1.0, 0.0))
                    vt_ref[2 * j, :, pl.ds(r0, TQ)] = ve.astype(BF16).astype(F32)
                    vo = qv[D + 40 * j + 16:D + 40 * j + 40]
                    vo = jnp.where(r24 >= 4, vo, jnp.where(r24 == 0, 1.0, 0.0))
                    vt_ref[2 * j + 1, :, pl.ds(r0, TQ)] = vo.astype(BF16).astype(F32)
                return carry

            with scope("p_qv"):
                lax.fori_loop(0, NQ, qv_step, 0)

            with scope("first_a"):
                for u in range(NH):
                    m8 = None
                    for c in range(NCK):
                        m8 = scores_mxu(u, u, c * CK, CK, m8)
                    finish_m(m8, u)
                for u in range(NH - 1):
                    prep_qb(NH + u, u)

        r8q = lax.broadcasted_iota(jnp.int32, (8, TQ), 0)

        def group(j, carry, with_scores=True):
            h0 = NH * j
            n0 = i * H + h0
            ms = [m_ref[u] for u in range(NH)]
            acc = [None] * NH
            for u in range(NH):
                m8 = None
                if with_scores and u == NH - 1:
                    prep_qb(n0 + NH + u, u)
                for c in range(NCK):
                    acc[u] = softmax_pv(h0 + u, u, ms[u], c, acc[u])
                    if with_scores:
                        r0 = c * CK + (16 if c in OFF else 0)
                        m8 = scores_mxu(n0 + NH + u, u, r0, (c + 1) * CK - r0, m8)
                        if c in OFF:
                            k = OFF.index(c)
                            for p in (2 * k, 2 * k + 1):
                                m8 = scores_vpu(n0 + NH + u, u, p, m8)
                if with_scores:
                    finish_m(m8, u)
                    if u < NH - 1:
                        prep_qb(n0 + 2 * NH + u, u)
            for u in range(0, NH, 2):
                oe = acc[u] * (1.0 / acc[u][20:21])
                oo = acc[u + 1] * (1.0 / acc[u + 1][0:1])
                base = j * (DH * NH) + DH * u
                if not isinstance(base, int):
                    base = pl.multiple_of(base, 8)
                ot_ref[pl.ds(base, 16), :] = oe[:16]
                ot_ref[pl.ds(base + 16, 8), :] = jnp.where(r8q < 4, oe[16:24], oo[:8])
                ot_ref[pl.ds(base + 24, 16), :] = oo[8:24]
            return carry

        with scope("attn_loop"):
            ngrp = jnp.where(i == NQ - 1, NGRP - 1, NGRP)
            lax.fori_loop(0, ngrp, group, 0)

        @pl.when(i == NQ - 1)
        def _():
            with scope("b_tail"):
                group(NGRP - 1, 0, with_scores=False)

        @pl.when(i == 0)
        def _():
            wo_copy.wait()
            w1_copy.wait()
            w2_copy.wait()

        with scope("epilogue"):
            R = TQ // ESPLIT
            hs = []
            for t in range(ESPLIT):
                o = ot_ref[:, pl.ds(t * R, R)].T.astype(BF16)
                r0 = pl.multiple_of(i * TQ + t * R, R)
                hs.append(x_ref[pl.ds(r0, R), :].astype(F32) + jnp.dot(
                    o, wo_ref[...], preferred_element_type=F32))
            acts = []
            for t in range(ESPLIT):
                hn = _ln(hs[t]).astype(BF16)
                a = (jnp.dot(hn, w1_ref[...], preferred_element_type=F32)
                     + b1_ref[...].astype(F32)[None, :])
                acts.append(_gelu(a).astype(BF16))
            for t in range(ESPLIT):
                y = (jnp.dot(acts[t], w2_ref[...], preferred_element_type=F32)
                     + b2_ref[...].astype(F32)[None, :])
                o_ref[pl.ds(t * R, R), :] = (hs[t] + y).astype(o_ref.dtype)

    return kernel


def build(NH=4, ESPLIT=2, OFF=(0, 2, 4, 6, 8, 10, 12, 14),
          XCH=((0, 256), (256, 512), (512, 1024), (1024, 2048)), PROF=False):
    OFF = list(OFF)
    NV = 16 * len(OFF)

    def fn(A_x, A_wqkv, A_wo, B_x, B_w1, B_b1, B_w2, B_b2):
        x = A_x.reshape(S, D)
        hbm = pl.BlockSpec(memory_space=pl.ANY)
        out = pl.pallas_call(
            _make_kernel(NH, ESPLIT, OFF, XCH, PROF),
            grid=(NQ,),
            in_specs=[hbm, hbm, hbm, hbm, pl.BlockSpec((F,), lambda i: (0,)),
                      hbm, pl.BlockSpec((D,), lambda i: (0,))],
            out_specs=pl.BlockSpec((TQ, D), lambda i: (i, 0)),
            out_shape=jax.ShapeDtypeStruct((S, D), BF16),
            scratch_shapes=[
                pltpu.VMEM((S, D), BF16),
                pltpu.VMEM((D, D), BF16),
                pltpu.VMEM((2, D, D), BF16),
                pltpu.VMEM((D, D), BF16),
                pltpu.VMEM((D, F), BF16),
                pltpu.VMEM((F, D), BF16),
                pltpu.VMEM((S, D), BF16),
                pltpu.VMEM((2 * D, D), BF16),
                pltpu.VMEM((NPAIR, S // 2, 128), U32),
                pltpu.VMEM((NPAIR, NQ, 40, TQ), U32),
                pltpu.VMEM((H, 24, S), F32),
                pltpu.VMEM((NH, S, TQ), F32),
                pltpu.VMEM((NH, 8, TQ), F32),
                pltpu.VMEM((D, TQ), F32),
                pltpu.VMEM((NPAIR, NV, 128), U32),
                pltpu.VMEM((H, DH, NV, 128), F32),
                pltpu.VMEM((NPAIR, NQ, 40, TQ), F32),
                pltpu.VMEM((NH, DH, 8, TQ), F32),
                pltpu.VMEM((24, TQ), F32),
                pltpu.SemaphoreType.DMA((len(XCH),)),
                pltpu.SemaphoreType.DMA((6,)),
            ],
            compiler_params=pltpu.CompilerParams(
                dimension_semantics=("arbitrary",),
                vmem_limit_bytes=120 * 1024 * 1024),
        )(x, A_wqkv, A_wo, B_w1, B_b1, B_w2, B_b2)
        return out.reshape(1, S, D)

    return jax.jit(fn)


_FN = build()


@jax.jit
def pallas_sequential_preLN__softmax_full_mha__dense_activation_gelu__prompt_kernel(
    A_x: jax.Array,
    A_wqkv: jax.Array,
    A_wo: jax.Array,
    B_x: jax.Array,
    B_w1: jax.Array,
    B_b1: jax.Array,
    B_w2: jax.Array,
    B_b2: jax.Array,
):
    return _FN(A_x, A_wqkv, A_wo, B_x, B_w1, B_b1, B_w2, B_b2)
```

```python
import math

import jax
import jax.numpy as jnp
from jax import lax
import jax.experimental.pallas as pl
import jax.experimental.pallas.tpu as pltpu

S = 2048
D = 640
H = 32
DH = 20
F = 1536
EPS = 1e-5
NG = D // 128
NPAIR = H // 2
LOG2E = 1.4426950408889634

F32 = jnp.float32
BF16 = jnp.bfloat16
U32 = jnp.uint32

TQ = 512
CK = 128
NQ = S // TQ
NCK = S // CK
NT = TQ // 128


def _ln(x):
    m = jnp.mean(x, axis=-1, keepdims=True)
    xc = x - m
    v = jnp.mean(xc * xc, axis=-1, keepdims=True)
    return xc * lax.rsqrt(v + EPS)


def _gelu(x):
    c = math.sqrt(2.0 / math.pi)
    inner = x * (c + (c * 0.044715) * (x * x))
    return x * (0.5 + 0.5 * jnp.tanh(inner))


class _NoScope:
    def __enter__(self):
        return self

    def __exit__(self, *a):
        return False


def _make_kernel(NH, ESPLIT, OFF, XCH, PROF, NSUB, POS0, PEND):
    NGRP = H // NH
    NOFF = len(OFF)
    NV = 16 * NOFF
    HPI = H // NQ
    scope = jax.named_scope if PROF else (lambda name: _NoScope())

    def kernel(x_hbm, wqkv_hbm, wo_hbm, w1_hbm, b1_ref, w2_hbm, b2_ref, o_ref,
               x_ref, wk_ref, wqv_ref, wo_ref, w1_ref, w2_ref,
               xn_ref, wt_ref, kp_ref, qh_ref, vt_ref, s_ref, m_ref, ot_ref,
               kw_ref, kb_ref, qth_ref, qb_ref, zero_ref, xsem, wsem):
        i = pl.program_id(0)

        def x_copy(r):
            a, b = XCH[r]
            return pltpu.make_async_copy(
                x_hbm.at[pl.ds(a, b - a), :], x_ref.at[pl.ds(a, b - a), :],
                xsem.at[r])

        wk_copy = pltpu.make_async_copy(wqkv_hbm.at[:, pl.ds(D, D)], wk_ref, wsem.at[0])
        wq_copy = pltpu.make_async_copy(wqkv_hbm.at[:, pl.ds(0, D)], wqv_ref.at[0], wsem.at[1])
        wv_copy = pltpu.make_async_copy(wqkv_hbm.at[:, pl.ds(2 * D, D)], wqv_ref.at[1], wsem.at[2])
        wo_copy = pltpu.make_async_copy(wo_hbm, wo_ref, wsem.at[3])
        w1_copy = pltpu.make_async_copy(w1_hbm, w1_ref, wsem.at[4])
        w2_copy = pltpu.make_async_copy(w2_hbm, w2_ref, wsem.at[5])

        def split_n(n):
            if isinstance(n, int):
                return n % H, min(n // H, NQ - 1)
            return n % H, jnp.minimum(n // H, NQ - 1)

        def prep_qb(n, u):
            h, qb = split_n(n)
            e = u % 2
            for a in range(2 * e, 2 * e + 3):
                q8 = qth_ref[h // 2, qb, pl.ds(8 * a, 8), :]
                for r in range(8):
                    d = 8 * a + r - DH * e
                    if 0 <= d < DH:
                        qb_ref[u, d] = jnp.broadcast_to(q8[r:r + 1], (8, TQ))

        def scores_mxu(n, u, r0, nr, m8, hook=None):
            h, qb = split_n(n)
            e = u % 2
            kd = 48 if e else 32
            k = pltpu.bitcast(kp_ref[h // 2, pl.ds(r0 // 2, nr // 2), :], BF16)
            q = pltpu.bitcast(qh_ref[h // 2, qb, pl.ds(16 * e, kd // 2), :], BF16)
            s = jnp.dot(k[:, :kd], q, preferred_element_type=F32)
            s_ref[u, pl.ds(r0, nr), :] = s
            if hook is None:
                pm = jnp.max(s.reshape(nr // 8, 8, TQ), axis=0)
                return pm if m8 is None else jnp.maximum(m8, pm)
            ng = nr // 8
            for qd in range(NSUB):
                a, b = (qd * ng) // NSUB, ((qd + 1) * ng) // NSUB
                pm = jnp.max(s[a * 8:b * 8].reshape(b - a, 8, TQ), axis=0)
                m8 = pm if m8 is None else jnp.maximum(m8, pm)
                m8 = hook(qd, m8)
            return m8

        def scores_vpu(n, u, p, m8):
            h, _ = split_n(n)
            acc = [None] * NT
            for jd in (range(DH // 2) if p % 2 == 0 else range(DH // 2 - 1, -1, -1)):
                lo = kb_ref[h, jd, pl.ds(p * 8, 8), :]
                hi = kb_ref[h, jd + DH // 2, pl.ds(p * 8, 8), :]
                for t in range(NT):
                    a = lo * qb_ref[u, jd, :, pl.ds(t * 128, 128)]
                    acc[t] = a if acc[t] is None else acc[t] + a
                    acc[t] = acc[t] + hi * qb_ref[u, jd + DH // 2, :, pl.ds(t * 128, 128)]
            row = OFF[p // 2] * CK + (p % 2) * 8
            for t in range(NT):
                s_ref[u, pl.ds(row, 8), pl.ds(t * 128, 128)] = acc[t]
            return jnp.maximum(m8, jnp.concatenate(acc, axis=1))

        def finish_m(m8, u):
            m = jnp.max(m8, axis=0, keepdims=True)
            m_ref[u] = jnp.broadcast_to(m, (8, TQ))

        def softmax_pv(h, u, m, c, acc):
            s = s_ref[u, pl.ds(c * CK, CK), :].reshape(CK // 8, 8, TQ)
            p = jnp.exp2(s - m[None]).reshape(CK, TQ)
            o = jnp.dot(vt_ref[h, :, pl.ds(c * CK, CK)], p,
                        preferred_element_type=F32)
            if acc is None:
                return (zero_ref[...] + o) if u > 0 else o
            return acc + o

        def ln_rows(a, b):
            for r0 in range(a, b, 256):
                xn_ref[pl.ds(r0, 256), :] = _ln(
                    x_ref[pl.ds(r0, 256), :].astype(F32)).astype(BF16)

        def kproj_rows(a, b):
            lane = lax.broadcasted_iota(jnp.int32, (128, 128), 1)
            for r0 in range(a, b, 256):
                k = jnp.dot(xn_ref[pl.ds(r0, 256), :], wk_ref[...],
                            preferred_element_type=F32)
                ku = pltpu.bitcast(k.astype(BF16), U32)
                for j in range(NPAIR):
                    start = 2 * DH * j
                    g0, g1 = start // 128, (start + 2 * DH - 1) // 128
                    kk = ku[:, g0 * 128:(g0 + 1) * 128]
                    if g1 != g0:
                        kk = jnp.where(lane >= 64, kk, ku[:, g1 * 128:(g1 + 1) * 128])
                    sh = (128 - start % 128) % 128
                    if sh:
                        kk = pltpu.roll(kk, sh, 1)
                    kp_ref[j, pl.ds(r0 // 2, 128), :] = kk

        def build_kw():
            for j in range(NPAIR):
                ku = jnp.concatenate(
                    [kp_ref[j, pl.ds(c * CK // 2, 8), :] for c in OFF], axis=0)
                kk = pltpu.bitcast(ku, BF16).astype(F32)
                kb = pltpu.bitcast(kk, U32)
                kw_ref[j] = ((pltpu.roll(kb, 128 - DH // 2, 1) & jnp.uint32(0xFFFF0000))
                             | (kb >> 16))

        @pl.when(i == 0)
        def _prologue():
            with scope("p_k"):
                x_copy(0).start()
                wk_copy.start()
                zero_ref[...] = jnp.zeros((24, TQ), F32)
                x_copy(1).start()
                x_copy(0).wait()
                x_copy(2).start()
                ln_rows(*XCH[0])
                wk_copy.wait()
                x_copy(1).wait()
                x_copy(3).start()
                ln_rows(*XCH[1])
                kproj_rows(*XCH[0])
                x_copy(2).wait()
                wq_copy.start()
                wv_copy.start()
                ln_rows(*XCH[2])
                kproj_rows(*XCH[1])
                x_copy(3).wait()
                ln_rows(*XCH[3])
                kproj_rows(*XCH[2])
                wq_copy.wait()
                wv_copy.wait()
                wo_copy.start()
                w1_copy.start()
                w2_copy.start()
                kproj_rows(*XCH[3])
                build_kw()
                for t in range(2):
                    for b in range(NG):
                        wt_ref[pl.ds(t * D + b * 128, 128), :] = (
                            wqv_ref[t, :, pl.ds(b * 128, 128)].astype(F32).T.astype(BF16))

            qscale = (DH ** -0.5) * LOG2E
            r24 = lax.broadcasted_iota(jnp.int32, (24, TQ), 0)
            r32 = lax.broadcasted_iota(jnp.int32, (32, TQ), 0)

            def qv_step(r, carry):
                r0 = pl.multiple_of(r * TQ, TQ)
                for hh in range(HPI):
                    kw = kw_ref[r * (HPI // 2) + hh // 2]
                    for jd in range(DH // 2):
                        l = DH * (hh % 2) + jd
                        w = jnp.broadcast_to(kw[:, l:l + 1], (NV, 128))
                        kb_ref[r * HPI + hh, jd] = pltpu.bitcast(w << 16, F32)
                        kb_ref[r * HPI + hh, jd + DH // 2] = pltpu.bitcast(
                            w & jnp.uint32(0xFFFF0000), F32)
                qv = lax.dot_general(wt_ref[...], xn_ref[pl.ds(r0, TQ), :],
                                     (((1,), (1,)), ((), ())),
                                     preferred_element_type=F32)
                zero16 = jnp.zeros((8, TQ), U32)
                for j in range(NPAIR):
                    q = qv[40 * j:40 * j + 48] * qscale
                    qe = jnp.where(r32 < DH, q[:32], 0.0).astype(BF16)
                    qo = jnp.where((r32 >= 4) & (r32 < 24), q[16:48], 0.0).astype(BF16)
                    qh_ref[j, r, pl.ds(0, 16), :] = pltpu.bitcast(qe, U32)
                    qh_ref[j, r, pl.ds(16, 8), :] = zero16
                    qh_ref[j, r, pl.ds(24, 16), :] = pltpu.bitcast(qo, U32)
                    qth_ref[j, r] = q[:40].astype(BF16).astype(F32)
                for j in range(NPAIR):
                    ve = qv[D + 40 * j:D + 40 * j + 24]
                    ve = jnp.where(r24 < DH, ve, jnp.where(r24 == DH, 1.0, 0.0))
                    vt_ref[2 * j, :, pl.ds(r0, TQ)] = ve.astype(BF16).astype(F32)
                    vo = qv[D + 40 * j + 16:D + 40 * j + 40]
                    vo = jnp.where(r24 >= 4, vo, jnp.where(r24 == 0, 1.0, 0.0))
                    vt_ref[2 * j + 1, :, pl.ds(r0, TQ)] = vo.astype(BF16).astype(F32)
                return carry

            with scope("p_qv"):
                lax.fori_loop(0, NQ, qv_step, 0)

            with scope("first_a"):
                for u in range(NH):
                    m8 = None
                    for c in range(NCK):
                        m8 = scores_mxu(u, u, c * CK, CK, m8)
                    finish_m(m8, u)
                for u in range(NH - 1):
                    prep_qb(NH + u, u)

        r8q = lax.broadcasted_iota(jnp.int32, (8, TQ), 0)

        def group(j, carry, with_scores=True):
            h0 = NH * j
            n0 = i * H + h0
            ms = [m_ref[u] for u in range(NH)]
            acc = [None] * NH
            for u in range(NH):
                m8 = None
                if with_scores and u == NH - 1:
                    prep_qb(n0 + NH + u, u)
                for c in range(NCK):
                    acc[u] = softmax_pv(h0 + u, u, ms[u], c, acc[u])
                    if with_scores:
                        r0 = c * CK + (16 if c in OFF else 0)
                        def hook(qd, m8, c=c, u=u):
                            for p in range(2 * NOFF):
                                pos = max(OFF[p // 2] * NSUB + NSUB - 1,
                                          POS0 + (p * (NCK * NSUB - POS0 - PEND)) // (2 * NOFF))
                                if pos == c * NSUB + qd:
                                    m8 = scores_vpu(n0 + NH + u, u, p, m8)
                            return m8
                        m8 = scores_mxu(n0 + NH + u, u, r0, (c + 1) * CK - r0, m8, hook)
                if with_scores:
                    finish_m(m8, u)
                    if u < NH - 1:
                        prep_qb(n0 + 2 * NH + u, u)
            for u in range(0, NH, 2):
                oe = acc[u] * (1.0 / acc[u][20:21])
                oo = acc[u + 1] * (1.0 / acc[u + 1][0:1])
                base = j * (DH * NH) + DH * u
                if not isinstance(base, int):
                    base = pl.multiple_of(base, 8)
                ot_ref[pl.ds(base, 16), :] = oe[:16]
                ot_ref[pl.ds(base + 16, 8), :] = jnp.where(r8q < 4, oe[16:24], oo[:8])
                ot_ref[pl.ds(base + 24, 16), :] = oo[8:24]
            return carry

        with scope("attn_loop"):
            ngrp = jnp.where(i == NQ - 1, NGRP - 1, NGRP)
            lax.fori_loop(0, ngrp, group, 0)

        @pl.when(i == NQ - 1)
        def _():
            with scope("b_tail"):
                group(NGRP - 1, 0, with_scores=False)

        @pl.when(i == 0)
        def _():
            wo_copy.wait()
            w1_copy.wait()
            w2_copy.wait()

        with scope("epilogue"):
            R = TQ // ESPLIT
            hs = []
            for t in range(ESPLIT):
                o = ot_ref[:, pl.ds(t * R, R)].T.astype(BF16)
                r0 = pl.multiple_of(i * TQ + t * R, R)
                hs.append(x_ref[pl.ds(r0, R), :].astype(F32) + jnp.dot(
                    o, wo_ref[...], preferred_element_type=F32))
            acts = []
            for t in range(ESPLIT):
                hn = _ln(hs[t]).astype(BF16)
                a = (jnp.dot(hn, w1_ref[...], preferred_element_type=F32)
                     + b1_ref[...].astype(F32)[None, :])
                acts.append(_gelu(a).astype(BF16))
            for t in range(ESPLIT):
                y = (jnp.dot(acts[t], w2_ref[...], preferred_element_type=F32)
                     + b2_ref[...].astype(F32)[None, :])
                o_ref[pl.ds(t * R, R), :] = (hs[t] + y).astype(o_ref.dtype)

    return kernel


def build(NH=4, ESPLIT=4, OFF=(0, 2, 4, 6, 8, 10, 12, 14),
          XCH=((0, 256), (256, 512), (512, 1024), (1024, 2048)), PROF=False, NSUB=4, POS0=3, PEND=0):
    OFF = list(OFF)
    NV = 16 * len(OFF)

    def fn(A_x, A_wqkv, A_wo, B_x, B_w1, B_b1, B_w2, B_b2):
        x = A_x.reshape(S, D)
        hbm = pl.BlockSpec(memory_space=pl.ANY)
        out = pl.pallas_call(
            _make_kernel(NH, ESPLIT, OFF, XCH, PROF, NSUB, POS0, PEND),
            grid=(NQ,),
            in_specs=[hbm, hbm, hbm, hbm, pl.BlockSpec((F,), lambda i: (0,)),
                      hbm, pl.BlockSpec((D,), lambda i: (0,))],
            out_specs=pl.BlockSpec((TQ, D), lambda i: (i, 0)),
            out_shape=jax.ShapeDtypeStruct((S, D), BF16),
            scratch_shapes=[
                pltpu.VMEM((S, D), BF16),
                pltpu.VMEM((D, D), BF16),
                pltpu.VMEM((2, D, D), BF16),
                pltpu.VMEM((D, D), BF16),
                pltpu.VMEM((D, F), BF16),
                pltpu.VMEM((F, D), BF16),
                pltpu.VMEM((S, D), BF16),
                pltpu.VMEM((2 * D, D), BF16),
                pltpu.VMEM((NPAIR, S // 2, 128), U32),
                pltpu.VMEM((NPAIR, NQ, 40, TQ), U32),
                pltpu.VMEM((H, 24, S), F32),
                pltpu.VMEM((NH, S, TQ), F32),
                pltpu.VMEM((NH, 8, TQ), F32),
                pltpu.VMEM((D, TQ), F32),
                pltpu.VMEM((NPAIR, NV, 128), U32),
                pltpu.VMEM((H, DH, NV, 128), F32),
                pltpu.VMEM((NPAIR, NQ, 40, TQ), F32),
                pltpu.VMEM((NH, DH, 8, TQ), F32),
                pltpu.VMEM((24, TQ), F32),
                pltpu.SemaphoreType.DMA((len(XCH),)),
                pltpu.SemaphoreType.DMA((6,)),
            ],
            compiler_params=pltpu.CompilerParams(
                dimension_semantics=("arbitrary",),
                vmem_limit_bytes=124 * 1024 * 1024),
        )(x, A_wqkv, A_wo, B_w1, B_b1, B_w2, B_b2)
        return out.reshape(1, S, D)

    return jax.jit(fn)


_FN = build(OFF=(0, 1, 2, 4, 5, 7, 8, 10, 11, 13))


@jax.jit
def pallas_sequential_preLN__softmax_full_mha__dense_activation_gelu__prompt_kernel(
    A_x: jax.Array,
    A_wqkv: jax.Array,
    A_wo: jax.Array,
    B_x: jax.Array,
    B_w1: jax.Array,
    B_b1: jax.Array,
    B_w2: jax.Array,
    B_b2: jax.Array,
):
    return _FN(A_x, A_wqkv, A_wo, B_x, B_w1, B_b1, B_w2, B_b2)
```

```python
import math

import jax
import jax.numpy as jnp
from jax import lax
import jax.experimental.pallas as pl
import jax.experimental.pallas.tpu as pltpu

S = 2048
D = 640
H = 32
DH = 20
F = 1536
EPS = 1e-5
NG = D // 128
NPAIR = H // 2
LOG2E = 1.4426950408889634

F32 = jnp.float32
BF16 = jnp.bfloat16
U32 = jnp.uint32

TQ = 512
CK = 128
NQ = S // TQ
NCK = S // CK
NT = TQ // 128


def _ln(x):
    m = jnp.mean(x, axis=-1, keepdims=True)
    xc = x - m
    v = jnp.mean(xc * xc, axis=-1, keepdims=True)
    return xc * lax.rsqrt(v + EPS)


def _gelu(x):
    c = math.sqrt(2.0 / math.pi)
    inner = x * (c + (c * 0.044715) * (x * x))
    return x * (0.5 + 0.5 * jnp.tanh(inner))


class _NoScope:
    def __enter__(self):
        return self

    def __exit__(self, *a):
        return False


def _make_kernel(NH, ESPLIT, OFF, XCH, NSUB, POS0, MODE, PROF):
    NGRP = H // NH
    NOFF = len(OFF)
    NV = 16 * NOFF
    NPC = 2 * NOFF
    HPI = H // NQ
    PPOS = [max(OFF[p // 2] * NSUB + NSUB - 1, POS0 + (p * (NCK * NSUB - POS0)) // NPC)
            for p in range(NPC)]
    scope = jax.named_scope if PROF else (lambda name: _NoScope())

    def kernel(x_hbm, wqkv_hbm, wo_hbm, w1_hbm, b1_hbm, w2_hbm, b2_hbm, o_hbm,
               x_ref, wk_ref, wqv_ref, wo_ref, w1_ref, w2_ref,
               xn_ref, wt_ref, kp_ref, qh_ref, vt_ref, s_ref, m_ref, ot_ref,
               kw_ref, kb_ref, qth_ref, qb_ref, zero_ref, o_ref, b1_ref, b2_ref, xsem, wsem, osem):
        i = pl.program_id(0)

        def x_copy(r):
            a, b = XCH[r]
            return pltpu.make_async_copy(
                x_hbm.at[pl.ds(a, b - a), :], x_ref.at[pl.ds(a, b - a), :],
                xsem.at[r])

        wk_copy = pltpu.make_async_copy(wqkv_hbm.at[:, pl.ds(D, D)], wk_ref, wsem.at[0])
        wq_copy = pltpu.make_async_copy(wqkv_hbm.at[:, pl.ds(0, D)], wqv_ref.at[0], wsem.at[1])
        wv_copy = pltpu.make_async_copy(wqkv_hbm.at[:, pl.ds(2 * D, D)], wqv_ref.at[1], wsem.at[2])
        wo_copy = pltpu.make_async_copy(wo_hbm, wo_ref, wsem.at[3])
        w1_copy = pltpu.make_async_copy(w1_hbm, w1_ref, wsem.at[4])
        w2_copy = pltpu.make_async_copy(w2_hbm, w2_ref, wsem.at[5])
        b1_copy = pltpu.make_async_copy(b1_hbm, b1_ref, wsem.at[6])
        b2_copy = pltpu.make_async_copy(b2_hbm, b2_ref, wsem.at[7])

        def split_n(n):
            if isinstance(n, int):
                return n % H, (n % H) // 2, min(n // H, NQ - 1)
            h = n & (H - 1)
            return h, h >> 1, jnp.minimum(n >> 5, NQ - 1)

        def prep_qb(hd, u):
            _, pr, qb = hd
            e = u % 2
            for a in range(2 * e, 2 * e + 3):
                q8 = qth_ref[pr, qb, pl.ds(8 * a, 8), :]
                for r in range(8):
                    d = 8 * a + r - DH * e
                    if 0 <= d < DH:
                        qb_ref[u, d] = jnp.broadcast_to(q8[r:r + 1], (8, TQ))

        def scores_vpu(hd, u, p, m8):
            kb = kb_ref[hd[0], :, pl.ds(p * 8, 8), :]
            kt = jnp.concatenate([kb] * NT, axis=2)
            q = qb_ref[u]
            if MODE == 0:
                sv = jnp.sum(kt * q, axis=0)
            else:
                sv = None
                for jd in range(DH // 2):
                    for d in (jd, jd + DH // 2):
                        a = kt[d] * q[d]
                        sv = a if sv is None else sv + a
            s_ref[u, pl.ds(OFF[p // 2] * CK + (p % 2) * 8, 8), :] = sv
            return jnp.maximum(m8, sv)

        def scores(hd, u, c, m8, offload):
            _, pr, qb = hd
            e = u % 2
            kd = 48 if e else 32
            r0 = c * CK + (16 if (offload and c in OFF) else 0)
            nr = (c + 1) * CK - r0
            k = pltpu.bitcast(kp_ref[pr, pl.ds(r0 // 2, nr // 2), :], BF16)
            q = pltpu.bitcast(qh_ref[pr, qb, pl.ds(16 * e, kd // 2), :], BF16)
            s = jnp.dot(k[:, :kd], q, preferred_element_type=F32)
            s_ref[u, pl.ds(r0, nr), :] = s
            nsub = NSUB if offload else 1
            ng = nr // 8
            for qd in range(nsub):
                a, b = (qd * ng) // nsub, ((qd + 1) * ng) // nsub
                pm = jnp.max(s[a * 8:b * 8].reshape(b - a, 8, TQ), axis=0)
                m8 = pm if m8 is None else jnp.maximum(m8, pm)
                if offload:
                    for p in range(NPC):
                        if PPOS[p] == c * NSUB + qd:
                            m8 = scores_vpu(hd, u, p, m8)
            return m8

        def finish_m(m8, u):
            m = jnp.max(m8, axis=0, keepdims=True)
            m_ref[u] = jnp.broadcast_to(m, (8, TQ))

        def softmax_pv(h, u, m, c, acc):
            s = s_ref[u, pl.ds(c * CK, CK), :].reshape(CK // 8, 8, TQ)
            p = jnp.exp2(s - m[None]).reshape(CK, TQ)
            o = jnp.dot(vt_ref[h, :, pl.ds(c * CK, CK)], p,
                        preferred_element_type=F32)
            if acc is None:
                return (zero_ref[...] + o) if u > 0 else o
            return acc + o

        def ln_rows(a, b):
            for r0 in range(a, b, 256):
                xn_ref[pl.ds(r0, 256), :] = _ln(
                    x_ref[pl.ds(r0, 256), :].astype(F32)).astype(BF16)

        def kproj_rows(a, b):
            lane = lax.broadcasted_iota(jnp.int32, (128, 128), 1)
            for r0 in range(a, b, 256):
                k = jnp.dot(xn_ref[pl.ds(r0, 256), :], wk_ref[...],
                            preferred_element_type=F32)
                ku = pltpu.bitcast(k.astype(BF16), U32)
                for j in range(NPAIR):
                    start = 2 * DH * j
                    g0, g1 = start // 128, (start + 2 * DH - 1) // 128
                    kk = ku[:, g0 * 128:(g0 + 1) * 128]
                    if g1 != g0:
                        kk = jnp.where(lane >= 64, kk, ku[:, g1 * 128:(g1 + 1) * 128])
                    sh = (128 - start % 128) % 128
                    if sh:
                        kk = pltpu.roll(kk, sh, 1)
                    kp_ref[j, pl.ds(r0 // 2, 128), :] = kk

        def build_kw():
            for j in range(NPAIR):
                ku = jnp.concatenate(
                    [kp_ref[j, pl.ds(c * CK // 2, 8), :] for c in OFF], axis=0)
                kk = pltpu.bitcast(ku, BF16).astype(F32)
                kb = pltpu.bitcast(kk, U32)
                kw_ref[j] = ((pltpu.roll(kb, 128 - DH // 2, 1) & jnp.uint32(0xFFFF0000))
                             | (kb >> 16))

        @pl.when(i == 0)
        def _prologue():
            with scope("p_k"):
                x_copy(0).start()
                wk_copy.start()
                zero_ref[...] = jnp.zeros((24, TQ), F32)
                x_copy(1).start()
                x_copy(0).wait()
                x_copy(2).start()
                ln_rows(*XCH[0])
                wk_copy.wait()
                x_copy(1).wait()
                x_copy(3).start()
                ln_rows(*XCH[1])
                kproj_rows(*XCH[0])
                x_copy(2).wait()
                wq_copy.start()
                wv_copy.start()
                ln_rows(*XCH[2])
                kproj_rows(*XCH[1])
                x_copy(3).wait()
                ln_rows(*XCH[3])
                kproj_rows(*XCH[2])
                wq_copy.wait()
                wv_copy.wait()
                wo_copy.start()
                w1_copy.start()
                w2_copy.start()
                b1_copy.start()
                b2_copy.start()
                kproj_rows(*XCH[3])
                build_kw()
                for t in range(2):
                    for b in range(NG):
                        wt_ref[pl.ds(t * D + b * 128, 128), :] = (
                            wqv_ref[t, :, pl.ds(b * 128, 128)].astype(F32).T.astype(BF16))

            qscale = (DH ** -0.5) * LOG2E
            r24 = lax.broadcasted_iota(jnp.int32, (24, TQ), 0)
            r32 = lax.broadcasted_iota(jnp.int32, (32, TQ), 0)

            def qv_step(r, carry):
                r0 = pl.multiple_of(r * TQ, TQ)
                for hh in range(HPI):
                    kw = kw_ref[r * (HPI // 2) + hh // 2]
                    for jd in range(DH // 2):
                        l = DH * (hh % 2) + jd
                        w = jnp.broadcast_to(kw[:, l:l + 1], (NV, 128))
                        kb_ref[r * HPI + hh, jd] = pltpu.bitcast(w << 16, F32)
                        kb_ref[r * HPI + hh, jd + DH // 2] = pltpu.bitcast(
                            w & jnp.uint32(0xFFFF0000), F32)
                qv = lax.dot_general(wt_ref[...], xn_ref[pl.ds(r0, TQ), :],
                                     (((1,), (1,)), ((), ())),
                                     preferred_element_type=F32)
                zero16 = jnp.zeros((8, TQ), U32)
                for j in range(NPAIR):
                    q = qv[40 * j:40 * j + 48] * qscale
                    qe = jnp.where(r32 < DH, q[:32], 0.0).astype(BF16)
                    qo = jnp.where((r32 >= 4) & (r32 < 24), q[16:48], 0.0).astype(BF16)
                    qh_ref[j, r, pl.ds(0, 16), :] = pltpu.bitcast(qe, U32)
                    qh_ref[j, r, pl.ds(16, 8), :] = zero16
                    qh_ref[j, r, pl.ds(24, 16), :] = pltpu.bitcast(qo, U32)
                    qth_ref[j, r] = q[:40].astype(BF16).astype(F32)
                for j in range(NPAIR):
                    ve = qv[D + 40 * j:D + 40 * j + 24]
                    ve = jnp.where(r24 < DH, ve, jnp.where(r24 == DH, 1.0, 0.0))
                    vt_ref[2 * j, :, pl.ds(r0, TQ)] = ve.astype(BF16).astype(F32)
                    vo = qv[D + 40 * j + 16:D + 40 * j + 40]
                    vo = jnp.where(r24 >= 4, vo, jnp.where(r24 == 0, 1.0, 0.0))
                    vt_ref[2 * j + 1, :, pl.ds(r0, TQ)] = vo.astype(BF16).astype(F32)
                return carry

            with scope("p_qv"):
                lax.fori_loop(0, NQ, qv_step, 0)

            with scope("first_a"):
                for u in range(NH):
                    m8 = None
                    for c in range(NCK):
                        m8 = scores(split_n(u), u, c, m8, False)
                    finish_m(m8, u)
                for u in range(NH - 1):
                    prep_qb(split_n(NH + u), u)

        r8q = lax.broadcasted_iota(jnp.int32, (8, TQ), 0)

        def group(j, carry, with_scores=True):
            h0 = NH * j
            n0 = i * H + h0
            ms = [m_ref[u] for u in range(NH)]
            acc = [None] * NH
            for u in range(NH):
                m8 = None
                if with_scores:
                    hd = split_n(n0 + NH + u)
                    if u == NH - 1:
                        prep_qb(hd, u)
                for c in range(NCK):
                    acc[u] = softmax_pv(h0 + u, u, ms[u], c, acc[u])
                    if with_scores:
                        m8 = scores(hd, u, c, m8, True)
                if with_scores:
                    finish_m(m8, u)
                    if u < NH - 1:
                        prep_qb(split_n(n0 + 2 * NH + u), u)
            for u in range(0, NH, 2):
                oe = acc[u] * (1.0 / acc[u][20:21])
                oo = acc[u + 1] * (1.0 / acc[u + 1][0:1])
                base = j * (DH * NH) + DH * u
                if not isinstance(base, int):
                    base = pl.multiple_of(base, 8)
                ot_ref[pl.ds(base, 16), :] = oe[:16]
                ot_ref[pl.ds(base + 16, 8), :] = jnp.where(r8q < 4, oe[16:24], oo[:8])
                ot_ref[pl.ds(base + 24, 16), :] = oo[8:24]
            return carry

        with scope("attn_loop"):
            ngrp = jnp.where(i == NQ - 1, NGRP - 1, NGRP)
            lax.fori_loop(0, ngrp, group, 0)

        @pl.when(i == NQ - 1)
        def _():
            with scope("b_tail"):
                group(NGRP - 1, 0, with_scores=False)

        @pl.when(i == 0)
        def _():
            wo_copy.wait()
            w1_copy.wait()
            w2_copy.wait()
            b1_copy.wait()
            b2_copy.wait()

        R = TQ // ESPLIT

        def out_copy(step, t):
            r0 = pl.multiple_of(step * TQ + t * R, R)
            return pltpu.make_async_copy(
                o_ref.at[pl.ds(t * R, R), :], o_hbm.at[pl.ds(r0, R), :], osem.at[t])

        @pl.when(i > 0)
        def _():
            for t in range(ESPLIT):
                out_copy(i - 1, t).wait()

        with scope("epilogue"):
            hs = []
            for t in range(ESPLIT):
                o = ot_ref[:, pl.ds(t * R, R)].T.astype(BF16)
                r0 = pl.multiple_of(i * TQ + t * R, R)
                hs.append(x_ref[pl.ds(r0, R), :].astype(F32) + jnp.dot(
                    o, wo_ref[...], preferred_element_type=F32))
            acts = []
            for t in range(ESPLIT):
                hn = _ln(hs[t]).astype(BF16)
                a = (jnp.dot(hn, w1_ref[...], preferred_element_type=F32)
                     + b1_ref[...].astype(F32)[None, :])
                acts.append(_gelu(a).astype(BF16))
            for t in range(ESPLIT):
                y = (jnp.dot(acts[t], w2_ref[...], preferred_element_type=F32)
                     + b2_ref[...].astype(F32)[None, :])
                o_ref[pl.ds(t * R, R), :] = (hs[t] + y).astype(o_ref.dtype)
                out_copy(i, t).start()

        @pl.when(i == NQ - 1)
        def _():
            for t in range(ESPLIT):
                out_copy(i, t).wait()

    return kernel


def build(NH=4, ESPLIT=4, OFF=(0, 1, 2, 4, 5, 7, 8, 10, 11, 13),
          XCH=((0, 256), (256, 512), (512, 1024), (1024, 2048)),
          NSUB=4, POS0=3, MODE=1, PROF=False, INTERPRET=False):
    OFF = list(OFF)
    NV = 16 * len(OFF)
    if INTERPRET:
        extra = dict(interpret=pltpu.InterpretParams(
            detect_races=True, uninitialized_memory="nan"))
    else:
        extra = dict(compiler_params=pltpu.CompilerParams(
            dimension_semantics=("arbitrary",),
            vmem_limit_bytes=124 * 1024 * 1024))

    def fn(A_x, A_wqkv, A_wo, B_x, B_w1, B_b1, B_w2, B_b2):
        x = A_x.reshape(S, D)
        hbm = pl.BlockSpec(memory_space=pl.ANY)
        out = pl.pallas_call(
            _make_kernel(NH, ESPLIT, OFF, XCH, NSUB, POS0, MODE, PROF),
            grid=(NQ,),
            in_specs=[hbm] * 7,
            out_specs=hbm,
            out_shape=jax.ShapeDtypeStruct((S, D), BF16),
            scratch_shapes=[
                pltpu.VMEM((S, D), BF16),
                pltpu.VMEM((D, D), BF16),
                pltpu.VMEM((2, D, D), BF16),
                pltpu.VMEM((D, D), BF16),
                pltpu.VMEM((D, F), BF16),
                pltpu.VMEM((F, D), BF16),
                pltpu.VMEM((S, D), BF16),
                pltpu.VMEM((2 * D, D), BF16),
                pltpu.VMEM((NPAIR, S // 2, 128), U32),
                pltpu.VMEM((NPAIR, NQ, 40, TQ), U32),
                pltpu.VMEM((H, 24, S), F32),
                pltpu.VMEM((NH, S, TQ), F32),
                pltpu.VMEM((NH, 8, TQ), F32),
                pltpu.VMEM((D, TQ), F32),
                pltpu.VMEM((NPAIR, NV, 128), U32),
                pltpu.VMEM((H, DH, NV, 128), F32),
                pltpu.VMEM((NPAIR, NQ, 40, TQ), F32),
                pltpu.VMEM((NH, DH, 8, TQ), F32),
                pltpu.VMEM((24, TQ), F32),
                pltpu.VMEM((TQ, D), BF16),
                pltpu.VMEM((F,), BF16),
                pltpu.VMEM((D,), BF16),
                pltpu.SemaphoreType.DMA((len(XCH),)),
                pltpu.SemaphoreType.DMA((8,)),
                pltpu.SemaphoreType.DMA((ESPLIT,)),
            ],
            **extra,
        )(x, A_wqkv, A_wo, B_w1, B_b1, B_w2, B_b2)
        return out.reshape(1, S, D)

    return jax.jit(fn)


_FN = build()


@jax.jit
def pallas_sequential_preLN__softmax_full_mha__dense_activation_gelu__prompt_kernel(
    A_x: jax.Array,
    A_wqkv: jax.Array,
    A_wo: jax.Array,
    B_x: jax.Array,
    B_w1: jax.Array,
    B_b1: jax.Array,
    B_w2: jax.Array,
    B_b2: jax.Array,
):
    return _FN(A_x, A_wqkv, A_wo, B_x, B_w1, B_b1, B_w2, B_b2)
```

```python
import math

import jax
import jax.numpy as jnp
from jax import lax
import jax.experimental.pallas as pl
import jax.experimental.pallas.tpu as pltpu

S = 2048
D = 640
H = 32
DH = 20
F = 1536
EPS = 1e-5
NG = D // 128
NPAIR = H // 2
LOG2E = 1.4426950408889634

F32 = jnp.float32
BF16 = jnp.bfloat16
U32 = jnp.uint32

TQ = 512
CK = 128
NQ = S // TQ
NCK = S // CK
NT = TQ // 128
NH = 4
NGRP = H // NH
ESPLIT = 4
R = TQ // ESPLIT
QSPLIT = 16
KM = 128
LM = 128
HPI = H // NQ
XCH = ((0, 256), (256, 512), (512, 1024), (1024, 2048))
OFF = [0, 1, 2, 4, 5, 7, 8, 10, 11, 13]
NV = 16 * len(OFF)
NPC = 2 * len(OFF)
NSUB = 4
PPOS = [max(OFF[p // 2] * NSUB + NSUB - 1, 3 + (p * (NCK * NSUB - 3)) // NPC)
        for p in range(NPC)]


def _ln(x):
    m = jnp.mean(x, axis=-1, keepdims=True)
    xc = x - m
    v = jnp.mean(xc * xc, axis=-1, keepdims=True)
    return xc * lax.rsqrt(v + EPS)


def _gelu(x):
    c = math.sqrt(2.0 / math.pi)
    inner = x * (c + (c * 0.044715) * (x * x))
    return x * (0.5 + 0.5 * jnp.tanh(inner))


def _kernel(x_hbm, wqkv_hbm, wo_hbm, w1_hbm, b1_hbm, w2_hbm, b2_hbm, o_hbm,
            x_ref, wk_ref, wqv_ref, wo_ref, w1_ref, w2_ref,
            xn_ref, wt_ref, kp_ref, qh_ref, vt_ref, s_ref, m_ref, ot_ref,
            kw_ref, kb_ref, qth_ref, qb_ref, zero_ref, o_ref, b1_ref, b2_ref,
            xsem, wsem, osem):
    i = pl.program_id(0)

    def x_copy(r):
        a, b = XCH[r]
        return pltpu.make_async_copy(
            x_hbm.at[pl.ds(a, b - a), :], x_ref.at[pl.ds(a, b - a), :], xsem.at[r])

    wk_copy = pltpu.make_async_copy(wqkv_hbm.at[:, pl.ds(D, D)], wk_ref, wsem.at[0])
    wq_copy = pltpu.make_async_copy(wqkv_hbm.at[:, pl.ds(0, D)], wqv_ref.at[0], wsem.at[1])
    wv_copy = pltpu.make_async_copy(wqkv_hbm.at[:, pl.ds(2 * D, D)], wqv_ref.at[1], wsem.at[2])
    late_copies = [
        pltpu.make_async_copy(wo_hbm, wo_ref, wsem.at[3]),
        pltpu.make_async_copy(w1_hbm, w1_ref, wsem.at[4]),
        pltpu.make_async_copy(w2_hbm, w2_ref, wsem.at[5]),
        pltpu.make_async_copy(b1_hbm, b1_ref, wsem.at[6]),
        pltpu.make_async_copy(b2_hbm, b2_ref, wsem.at[7]),
    ]

    def out_copy(step, t):
        r0 = pl.multiple_of(step * TQ + t * R, R)
        return pltpu.make_async_copy(
            o_ref.at[pl.ds(t * R, R), :], o_hbm.at[pl.ds(r0, R), :], osem.at[t])

    def split_n(n):
        if isinstance(n, int):
            return n % H, (n % H) // 2, min(n // H, NQ - 1)
        h = n & (H - 1)
        return h, h >> 1, jnp.minimum(n >> 5, NQ - 1)

    def prep_qb(hd, u):
        _, pr, qb = hd
        e = u % 2
        for a in range(2 * e, 2 * e + 3):
            q8 = qth_ref[pr, qb, pl.ds(8 * a, 8), :]
            for r in range(8):
                d = 8 * a + r - DH * e
                if 0 <= d < DH:
                    qb_ref[u, d] = jnp.broadcast_to(q8[r:r + 1], (8, TQ))

    def scores_vpu(hd, u, p, m8):
        kb = kb_ref[hd[0], :, pl.ds(p * 8, 8), :]
        kt = jnp.concatenate([kb] * NT, axis=2)
        q = qb_ref[u]
        sv = None
        for jd in range(DH // 2):
            for d in (jd, jd + DH // 2):
                a = kt[d] * q[d]
                sv = a if sv is None else sv + a
        s_ref[u, pl.ds(OFF[p // 2] * CK + (p % 2) * 8, 8), :] = sv
        return jnp.maximum(m8, sv)

    def scores(hd, u, c, m8, offload):
        _, pr, qb = hd
        e = u % 2
        kd = 48 if e else 32
        r0 = c * CK + (16 if (offload and c in OFF) else 0)
        nr = (c + 1) * CK - r0
        k = pltpu.bitcast(kp_ref[pr, pl.ds(r0 // 2, nr // 2), :], BF16)
        q = pltpu.bitcast(qh_ref[pr, qb, pl.ds(16 * e, kd // 2), :], BF16)
        s = jnp.dot(k[:, :kd], q, preferred_element_type=F32)
        s_ref[u, pl.ds(r0, nr), :] = s
        nsub = NSUB if offload else 1
        ng = nr // 8
        for qd in range(nsub):
            a, b = (qd * ng) // nsub, ((qd + 1) * ng) // nsub
            pm = jnp.max(s[a * 8:b * 8].reshape(b - a, 8, TQ), axis=0)
            m8 = pm if m8 is None else jnp.maximum(m8, pm)
            if offload:
                for p in range(NPC):
                    if PPOS[p] == c * NSUB + qd:
                        m8 = scores_vpu(hd, u, p, m8)
        return m8

    def finish_m(m8, u):
        m = jnp.max(m8, axis=0, keepdims=True)
        m_ref[u] = jnp.broadcast_to(m, (8, TQ))

    def softmax_pv(h, u, m, c, acc):
        s = s_ref[u, pl.ds(c * CK, CK), :].reshape(CK // 8, 8, TQ)
        p = jnp.exp2(s - m[None]).reshape(CK, TQ)
        o = jnp.dot(vt_ref[h, :, pl.ds(c * CK, CK)], p, preferred_element_type=F32)
        if acc is None:
            return (zero_ref[...] + o) if u > 0 else o
        return acc + o

    def ln_rows(a, b):
        for r0 in range(a, b, LM):
            xn_ref[pl.ds(r0, LM), :] = _ln(
                x_ref[pl.ds(r0, LM), :].astype(F32)).astype(BF16)

    def kproj_rows(a, b):
        lane = lax.broadcasted_iota(jnp.int32, (KM // 2, 128), 1)
        for r0 in range(a, b, KM):
            k = jnp.dot(xn_ref[pl.ds(r0, KM), :], wk_ref[...],
                        preferred_element_type=F32)
            ku = pltpu.bitcast(k.astype(BF16), U32)
            for j in range(NPAIR):
                start = 2 * DH * j
                g0, g1 = start // 128, (start + 2 * DH - 1) // 128
                kk = ku[:, g0 * 128:(g0 + 1) * 128]
                if g1 != g0:
                    kk = jnp.where(lane >= 64, kk, ku[:, g1 * 128:(g1 + 1) * 128])
                sh = (128 - start % 128) % 128
                if sh:
                    kk = pltpu.roll(kk, sh, 1)
                kp_ref[j, pl.ds(r0 // 2, KM // 2), :] = kk

    def ln_and_kproj(lr, kr):
        ls = list(range(lr[0], lr[1], LM))
        ks = list(range(kr[0], kr[1], KM))
        for n, k0 in enumerate(ks):
            for l0 in ls[(n * len(ls)) // len(ks):((n + 1) * len(ls)) // len(ks)]:
                ln_rows(l0, l0 + LM)
            kproj_rows(k0, k0 + KM)

    def build_kw():
        for j in range(NPAIR):
            ku = jnp.concatenate(
                [kp_ref[j, pl.ds(c * CK // 2, 8), :] for c in OFF], axis=0)
            kk = pltpu.bitcast(ku, BF16).astype(F32)
            kb = pltpu.bitcast(kk, U32)
            kw_ref[j] = ((pltpu.roll(kb, 128 - DH // 2, 1) & jnp.uint32(0xFFFF0000))
                         | (kb >> 16))

    def build_kb(pr, e):
        kw = kw_ref[pr]
        for jd in range(DH // 2):
            l = DH * e + jd
            w = jnp.broadcast_to(kw[:, l:l + 1], (NV, 128))
            kb_ref[2 * pr + e, jd] = pltpu.bitcast(w << 16, F32)
            kb_ref[2 * pr + e, jd + DH // 2] = pltpu.bitcast(
                w & jnp.uint32(0xFFFF0000), F32)

    @pl.when(i == 0)
    def _prologue():
        x_copy(0).start()
        wk_copy.start()
        zero_ref[...] = jnp.zeros((24, TQ), F32)
        x_copy(1).start()
        x_copy(0).wait()
        x_copy(2).start()
        ln_rows(*XCH[0])
        wk_copy.wait()
        x_copy(1).wait()
        x_copy(3).start()
        ln_and_kproj(XCH[1], XCH[0])
        x_copy(2).wait()
        wq_copy.start()
        wv_copy.start()
        ln_and_kproj(XCH[2], XCH[1])
        x_copy(3).wait()
        ln_and_kproj(XCH[3], XCH[2])
        wq_copy.wait()
        wv_copy.wait()
        for cp in late_copies:
            cp.start()
        kproj_rows(*XCH[3])
        build_kw()
        for t in range(2):
            for b in range(NG):
                wt_ref[pl.ds(t * D + b * 128, 128), :] = (
                    wqv_ref[t, :, pl.ds(b * 128, 128)].astype(F32).T.astype(BF16))

        qscale = (DH ** -0.5) * LOG2E
        r24 = lax.broadcasted_iota(jnp.int32, (24, TQ), 0)
        r32 = lax.broadcasted_iota(jnp.int32, (32, TQ), 0)

        def qv_step(r, carry):
            r0 = pl.multiple_of(r * TQ, TQ)
            xn = xn_ref[pl.ds(r0, TQ), :]
            zero16 = jnp.zeros((8, TQ), U32)
            mr = 2 * D // QSPLIT
            pps = mr // (2 * DH)
            for b in range(QSPLIT):
                for hh in range((b * HPI) // QSPLIT, ((b + 1) * HPI) // QSPLIT):
                    build_kb(r * (HPI // 2) + hh // 2, hh % 2)
                qv = lax.dot_general(wt_ref[pl.ds(b * mr, mr), :], xn,
                                     (((1,), (1,)), ((), ())),
                                     preferred_element_type=F32)
                for jj in range(pps):
                    g = b * pps + jj
                    blk = qv[40 * jj:40 * jj + 40]
                    if g < NPAIR:
                        q = blk * qscale
                        qe = jnp.where(r32 < DH, q[:32], 0.0).astype(BF16)
                        qo = jnp.concatenate(
                            [jnp.where(r24 >= 4, q[16:40], 0.0),
                             jnp.zeros((8, TQ), F32)], axis=0).astype(BF16)
                        qh_ref[g, r, pl.ds(0, 16), :] = pltpu.bitcast(qe, U32)
                        qh_ref[g, r, pl.ds(16, 8), :] = zero16
                        qh_ref[g, r, pl.ds(24, 16), :] = pltpu.bitcast(qo, U32)
                        qth_ref[g, r] = q.astype(BF16).astype(F32)
                    else:
                        j = g - NPAIR
                        ve = jnp.where(r24 < DH, blk[:24], jnp.where(r24 == DH, 1.0, 0.0))
                        vt_ref[2 * j, :, pl.ds(r0, TQ)] = ve.astype(BF16).astype(F32)
                        vo = jnp.where(r24 >= 4, blk[16:40], jnp.where(r24 == 0, 1.0, 0.0))
                        vt_ref[2 * j + 1, :, pl.ds(r0, TQ)] = vo.astype(BF16).astype(F32)
            return carry

        lax.fori_loop(0, NQ, qv_step, 0)

        for u in range(NH):
            m8 = None
            for c in range(NCK):
                m8 = scores(split_n(u), u, c, m8, False)
            finish_m(m8, u)
            if u < NH - 1:
                prep_qb(split_n(NH + u), u)

    r8q = lax.broadcasted_iota(jnp.int32, (8, TQ), 0)

    def group(j, carry, with_scores=True):
        h0 = NH * j
        n0 = i * H + h0
        ms = [m_ref[u] for u in range(NH)]
        acc = [None] * NH
        for u in range(NH):
            m8 = None
            if with_scores:
                hd = split_n(n0 + NH + u)
                if u == NH - 1:
                    prep_qb(hd, u)
            for c in range(NCK):
                acc[u] = softmax_pv(h0 + u, u, ms[u], c, acc[u])
                if with_scores:
                    m8 = scores(hd, u, c, m8, True)
            if with_scores:
                finish_m(m8, u)
                if u < NH - 1:
                    prep_qb(split_n(n0 + 2 * NH + u), u)
        for u in range(0, NH, 2):
            oe = acc[u] * (1.0 / acc[u][20:21])
            oo = acc[u + 1] * (1.0 / acc[u + 1][0:1])
            base = j * (DH * NH) + DH * u
            if not isinstance(base, int):
                base = pl.multiple_of(base, 8)
            ot_ref[pl.ds(base, 16), :] = oe[:16]
            ot_ref[pl.ds(base + 16, 8), :] = jnp.where(r8q < 4, oe[16:24], oo[:8])
            ot_ref[pl.ds(base + 24, 16), :] = oo[8:24]
        return carry

    lax.fori_loop(0, jnp.where(i == NQ - 1, NGRP - 1, NGRP), group, 0)

    @pl.when(i == NQ - 1)
    def _():
        group(NGRP - 1, 0, with_scores=False)

    @pl.when(i == 0)
    def _():
        for cp in late_copies:
            cp.wait()

    @pl.when(i > 0)
    def _():
        for t in range(ESPLIT):
            out_copy(i - 1, t).wait()

    hs = []
    for t in range(ESPLIT):
        o = ot_ref[:, pl.ds(t * R, R)].T.astype(BF16)
        r0 = pl.multiple_of(i * TQ + t * R, R)
        hs.append(x_ref[pl.ds(r0, R), :].astype(F32) + jnp.dot(
            o, wo_ref[...], preferred_element_type=F32))
    acts = []
    for t in range(ESPLIT):
        hn = _ln(hs[t]).astype(BF16)
        a = (jnp.dot(hn, w1_ref[...], preferred_element_type=F32)
             + b1_ref[...].astype(F32)[None, :])
        acts.append(_gelu(a).astype(BF16))
    for t in range(ESPLIT):
        y = (jnp.dot(acts[t], w2_ref[...], preferred_element_type=F32)
             + b2_ref[...].astype(F32)[None, :])
        o_ref[pl.ds(t * R, R), :] = (hs[t] + y).astype(BF16)
        out_copy(i, t).start()

    @pl.when(i == NQ - 1)
    def _():
        for t in range(ESPLIT):
            out_copy(i, t).wait()


@jax.jit
def pallas_sequential_preLN__softmax_full_mha__dense_activation_gelu__prompt_kernel(
    A_x: jax.Array,
    A_wqkv: jax.Array,
    A_wo: jax.Array,
    B_x: jax.Array,
    B_w1: jax.Array,
    B_b1: jax.Array,
    B_w2: jax.Array,
    B_b2: jax.Array,
):
    hbm = pl.BlockSpec(memory_space=pl.ANY)
    out = pl.pallas_call(
        _kernel,
        grid=(NQ,),
        in_specs=[hbm] * 7,
        out_specs=hbm,
        out_shape=jax.ShapeDtypeStruct((S, D), BF16),
        scratch_shapes=[
            pltpu.VMEM((S, D), BF16),
            pltpu.VMEM((D, D), BF16),
            pltpu.VMEM((2, D, D), BF16),
            pltpu.VMEM((D, D), BF16),
            pltpu.VMEM((D, F), BF16),
            pltpu.VMEM((F, D), BF16),
            pltpu.VMEM((S, D), BF16),
            pltpu.VMEM((2 * D, D), BF16),
            pltpu.VMEM((NPAIR, S // 2, 128), U32),
            pltpu.VMEM((NPAIR, NQ, 40, TQ), U32),
            pltpu.VMEM((H, 24, S), F32),
            pltpu.VMEM((NH, S, TQ), F32),
            pltpu.VMEM((NH, 8, TQ), F32),
            pltpu.VMEM((D, TQ), F32),
            pltpu.VMEM((NPAIR, NV, 128), U32),
            pltpu.VMEM((H, DH, NV, 128), F32),
            pltpu.VMEM((NPAIR, NQ, 40, TQ), F32),
            pltpu.VMEM((NH, DH, 8, TQ), F32),
            pltpu.VMEM((24, TQ), F32),
            pltpu.VMEM((TQ, D), BF16),
            pltpu.VMEM((F,), BF16),
            pltpu.VMEM((D,), BF16),
            pltpu.SemaphoreType.DMA((len(XCH),)),
            pltpu.SemaphoreType.DMA((8,)),
            pltpu.SemaphoreType.DMA((ESPLIT,)),
        ],
        compiler_params=pltpu.CompilerParams(
            dimension_semantics=("arbitrary",),
            vmem_limit_bytes=124 * 1024 * 1024),
    )(A_x.reshape(S, D), A_wqkv, A_wo, B_w1, B_b1, B_w2, B_b2)
    return out.reshape(1, S, D)
```

```python
import math

import jax
import jax.numpy as jnp
from jax import lax
import jax.experimental.pallas as pl
import jax.experimental.pallas.tpu as pltpu

S = 2048
D = 640
H = 32
DH = 20
F = 1536
EPS = 1e-5
NG = D // 128
NPAIR = H // 2
LOG2E = 1.4426950408889634

F32 = jnp.float32
BF16 = jnp.bfloat16
U32 = jnp.uint32

TQ = 512
CK = 128
NQ = S // TQ
NCK = S // CK
NT = TQ // 128
NH = 4
NGRP = H // NH
ESPLIT = 4
R = TQ // ESPLIT
QSPLIT = 16
KM = 128
LM = 128
HPI = H // NQ
XCH = ((0, 256), (256, 512), (512, 1024), (1024, 2048))
KB4 = 1152
LSPLIT = 1536
LLEAD = 384
OFF = [0, 1, 2, 4, 5, 7, 8, 10, 11, 13]
NV = 16 * len(OFF)
NPC = 2 * len(OFF)
NSUB = 4
PPOS = [max(OFF[p // 2] * NSUB + NSUB - 1, 3 + (p * (NCK * NSUB - 3)) // NPC)
        for p in range(NPC)]


def _ln(x):
    m = jnp.mean(x, axis=-1, keepdims=True)
    xc = x - m
    v = jnp.mean(xc * xc, axis=-1, keepdims=True)
    return xc * lax.rsqrt(v + EPS)


def _gelu(x):
    c = math.sqrt(2.0 / math.pi)
    inner = x * (c + (c * 0.044715) * (x * x))
    return x * (0.5 + 0.5 * jnp.tanh(inner))


def _kernel(x_hbm, wqkv_hbm, wo_hbm, w1_hbm, b1_hbm, w2_hbm, b2_hbm, o_hbm,
            x_ref, wk_ref, wqv_ref, wo_ref, w1_ref, w2_ref,
            xn_ref, wt_ref, kp_ref, qh_ref, vt_ref, s_ref, m_ref, ot_ref,
            kw_ref, kb_ref, qth_ref, qb_ref, zero_ref, kraw_ref, o_ref, b1_ref, b2_ref,
            xsem, wsem, osem):
    i = pl.program_id(0)

    def x_copy(r):
        a, b = XCH[r]
        return pltpu.make_async_copy(
            x_hbm.at[pl.ds(a, b - a), :], x_ref.at[pl.ds(a, b - a), :], xsem.at[r])

    wk_copy = pltpu.make_async_copy(wqkv_hbm.at[:, pl.ds(D, D)], wk_ref, wsem.at[0])
    wq_copy = pltpu.make_async_copy(wqkv_hbm.at[:, pl.ds(0, D)], wqv_ref.at[0], wsem.at[1])
    wv_copy = pltpu.make_async_copy(wqkv_hbm.at[:, pl.ds(2 * D, D)], wqv_ref.at[1], wsem.at[2])
    late_copies = [
        pltpu.make_async_copy(wo_hbm, wo_ref, wsem.at[3]),
        pltpu.make_async_copy(w1_hbm, w1_ref, wsem.at[4]),
        pltpu.make_async_copy(w2_hbm, w2_ref, wsem.at[5]),
        pltpu.make_async_copy(b1_hbm, b1_ref, wsem.at[6]),
        pltpu.make_async_copy(b2_hbm, b2_ref, wsem.at[7]),
    ]

    def out_copy(step, t):
        r0 = pl.multiple_of(step * TQ + t * R, R)
        return pltpu.make_async_copy(
            o_ref.at[pl.ds(t * R, R), :], o_hbm.at[pl.ds(r0, R), :], osem.at[t])

    def split_n(n):
        if isinstance(n, int):
            return n % H, (n % H) // 2, min(n // H, NQ - 1)
        h = n & (H - 1)
        return h, h >> 1, jnp.minimum(n >> 5, NQ - 1)

    def prep_qb(hd, u):
        _, pr, qb = hd
        e = u % 2
        for a in range(2 * e, 2 * e + 3):
            q8 = qth_ref[pr, qb, pl.ds(8 * a, 8), :]
            for r in range(8):
                d = 8 * a + r - DH * e
                if 0 <= d < DH:
                    qb_ref[u, d] = jnp.broadcast_to(q8[r:r + 1], (8, TQ))

    def prep_part(hd, u, a, t, anchor):
        _, pr, qb = hd
        e = u % 2
        a = a + 2 * e
        q8 = qth_ref[pr, qb, pl.ds(8 * a, 8), pl.ds(t * 128, 128)]
        an = anchor[:, t * 128:(t + 1) * 128]
        q8 = jnp.where(an != an, an, q8)
        for r in range(8):
            d = 8 * a + r - DH * e
            if 0 <= d < DH:
                qb_ref[u, d, :, pl.ds(t * 128, 128)] = jnp.broadcast_to(q8[r:r + 1], (8, 128))

    def scores_vpu(hd, u, p, m8):
        kb = kb_ref[hd[0], :, pl.ds(p * 8, 8), :]
        kt = jnp.concatenate([kb] * NT, axis=2)
        q = qb_ref[u]
        sv = None
        for jd in range(DH // 2):
            for d in (jd, jd + DH // 2):
                a = kt[d] * q[d]
                sv = a if sv is None else sv + a
        s_ref[u, pl.ds(OFF[p // 2] * CK + (p % 2) * 8, 8), :] = sv
        return jnp.maximum(m8, sv)

    def scores(hd, u, c, m8, offload):
        _, pr, qb = hd
        e = u % 2
        kd = 48 if e else 32
        r0 = c * CK + (16 if (offload and c in OFF) else 0)
        nr = (c + 1) * CK - r0
        k = pltpu.bitcast(kp_ref[pr, pl.ds(r0 // 2, nr // 2), :], BF16)
        q = pltpu.bitcast(qh_ref[pr, qb, pl.ds(16 * e, kd // 2), :], BF16)
        s = jnp.dot(k[:, :kd], q, preferred_element_type=F32)
        s_ref[u, pl.ds(r0, nr), :] = s
        nsub = NSUB if offload else 1
        ng = nr // 8
        for qd in range(nsub):
            a, b = (qd * ng) // nsub, ((qd + 1) * ng) // nsub
            pm = jnp.max(s[a * 8:b * 8].reshape(b - a, 8, TQ), axis=0)
            m8 = pm if m8 is None else jnp.maximum(m8, pm)
            if offload:
                for p in range(NPC):
                    if PPOS[p] == c * NSUB + qd:
                        m8 = scores_vpu(hd, u, p, m8)
        return m8

    def finish_m(m8, u):
        m = jnp.max(m8, axis=0, keepdims=True)
        m_ref[u] = jnp.broadcast_to(m, (8, TQ))

    def softmax_pv(h, u, m, c, acc):
        s = s_ref[u, pl.ds(c * CK, CK), :].reshape(CK // 8, 8, TQ)
        p = jnp.exp2(s - m[None]).reshape(CK, TQ)
        o = jnp.dot(vt_ref[h, :, pl.ds(c * CK, CK)], p, preferred_element_type=F32)
        if acc is None:
            return (zero_ref[...] + o) if u > 0 else o
        return acc + o

    def ln_rows(a, b):
        for r0 in range(a, b, LM):
            xn_ref[pl.ds(r0, LM), :] = _ln(
                x_ref[pl.ds(r0, LM), :].astype(F32)).astype(BF16)

    def store_pairs(ku, r0):
        lane = lax.broadcasted_iota(jnp.int32, (KM // 2, 128), 1)
        for j in range(NPAIR):
            start = 2 * DH * j
            g0, g1 = start // 128, (start + 2 * DH - 1) // 128
            kk = ku[:, g0 * 128:(g0 + 1) * 128]
            if g1 != g0:
                kk = jnp.where(lane >= 64, kk, ku[:, g1 * 128:(g1 + 1) * 128])
            sh = (128 - start % 128) % 128
            if sh:
                kk = pltpu.roll(kk, sh, 1)
            kp_ref[j, pl.ds(r0 // 2, KM // 2), :] = kk

    def kproj_rows(a, b, defer_last=None):
        for r0 in range(a, b, KM):
            k = jnp.dot(xn_ref[pl.ds(r0, KM), :], wk_ref[...],
                        preferred_element_type=F32)
            ku = pltpu.bitcast(k.astype(BF16), U32)
            if defer_last is not None and r0 + KM == b:
                kraw_ref[defer_last] = ku
            else:
                store_pairs(ku, r0)

    def ln_and_kproj(lr, kr, slot):
        if slot > 0:
            store_pairs(kraw_ref[slot - 1], kr[0] - KM)
        ls = list(range(lr[0], lr[1], LM))
        ks = list(range(kr[0], kr[1], KM))
        for n, k0 in enumerate(ks):
            for l0 in ls[(n * len(ls)) // len(ks):((n + 1) * len(ls)) // len(ks)]:
                ln_rows(l0, l0 + LM)
            kproj_rows(k0, k0 + KM, slot if k0 + KM == kr[1] else None)

    def build_kw():
        for j in range(NPAIR):
            ku = jnp.concatenate(
                [kp_ref[j, pl.ds(c * CK // 2, 8), :] for c in OFF], axis=0)
            kk = pltpu.bitcast(ku, BF16).astype(F32)
            kb = pltpu.bitcast(kk, U32)
            kw_ref[j] = ((pltpu.roll(kb, 128 - DH // 2, 1) & jnp.uint32(0xFFFF0000))
                         | (kb >> 16))

    def build_kb(pr, e):
        kw = kw_ref[pr]
        for jd in range(DH // 2):
            l = DH * e + jd
            w = jnp.broadcast_to(kw[:, l:l + 1], (NV, 128))
            kb_ref[2 * pr + e, jd] = pltpu.bitcast(w << 16, F32)
            kb_ref[2 * pr + e, jd + DH // 2] = pltpu.bitcast(
                w & jnp.uint32(0xFFFF0000), F32)

    @pl.when(i == 0)
    def _prologue():
        x_copy(0).start()
        wk_copy.start()
        zero_ref[...] = jnp.zeros((24, TQ), F32)
        x_copy(1).start()
        x_copy(0).wait()
        x_copy(2).start()
        ln_rows(*XCH[0])
        wk_copy.wait()
        x_copy(1).wait()
        x_copy(3).start()
        ln_and_kproj(XCH[1], XCH[0], 0)
        x_copy(2).wait()
        wq_copy.start()
        wv_copy.start()
        ln_and_kproj(XCH[2], XCH[1], 1)
        x_copy(3).wait()
        ln_and_kproj((XCH[3][0], LSPLIT), (XCH[2][0], KB4), 2)
        wq_copy.wait()
        wv_copy.wait()
        for cp in late_copies:
            cp.start()
        store_pairs(kraw_ref[2], KB4 - KM)
        for t in range(2):
            for b in range(NG):
                wt_ref[pl.ds(t * D + b * 128, 128), :] = (
                    wqv_ref[t, :, pl.ds(b * 128, 128)].astype(F32).T.astype(BF16))
        for k0 in range(KB4, (OFF[-1] + 1) * CK, KM):
            if LSPLIT <= k0 + LLEAD < S:
                ln_rows(k0 + LLEAD, k0 + LLEAD + KM)
            kproj_rows(k0, k0 + KM)
        build_kw()
        kproj_rows((OFF[-1] + 1) * CK, S, 3)

        qscale = (DH ** -0.5) * LOG2E
        r24 = lax.broadcasted_iota(jnp.int32, (24, TQ), 0)
        r32 = lax.broadcasted_iota(jnp.int32, (32, TQ), 0)

        def qv_step(r, carry):
            r0 = pl.multiple_of(r * TQ, TQ)
            xn = xn_ref[pl.ds(r0, TQ), :]
            zero16 = jnp.zeros((8, TQ), U32)
            mr = 2 * D // QSPLIT
            pps = mr // (2 * DH)
            for b in range(QSPLIT):
                for hh in range((b * HPI) // QSPLIT, ((b + 1) * HPI) // QSPLIT):
                    build_kb(r * (HPI // 2) + hh // 2, hh % 2)
                qv = lax.dot_general(wt_ref[pl.ds(b * mr, mr), :], xn,
                                     (((1,), (1,)), ((), ())),
                                     preferred_element_type=F32)
                for jj in range(pps):
                    g = b * pps + jj
                    blk = qv[40 * jj:40 * jj + 40]
                    if g < NPAIR:
                        q = blk * qscale
                        qe = jnp.where(r32 < DH, q[:32], 0.0).astype(BF16)
                        qo = jnp.concatenate(
                            [jnp.where(r24 >= 4, q[16:40], 0.0),
                             jnp.zeros((8, TQ), F32)], axis=0).astype(BF16)
                        qh_ref[g, r, pl.ds(0, 16), :] = pltpu.bitcast(qe, U32)
                        qh_ref[g, r, pl.ds(16, 8), :] = zero16
                        qh_ref[g, r, pl.ds(24, 16), :] = pltpu.bitcast(qo, U32)
                        qth_ref[g, r] = q.astype(BF16).astype(F32)
                    else:
                        j = g - NPAIR
                        ve = jnp.where(r24 < DH, blk[:24], jnp.where(r24 == DH, 1.0, 0.0))
                        vt_ref[2 * j, :, pl.ds(r0, TQ)] = ve.astype(BF16).astype(F32)
                        vo = jnp.where(r24 >= 4, blk[16:40], jnp.where(r24 == 0, 1.0, 0.0))
                        vt_ref[2 * j + 1, :, pl.ds(r0, TQ)] = vo.astype(BF16).astype(F32)
            return carry

        lax.fori_loop(0, NQ, qv_step, 0)

        store_pairs(kraw_ref[3], S - KM)
        for u in range(NH):
            m8 = None
            for c in range(NCK):
                m8 = scores(split_n(u), u, c, m8, False)
            finish_m(m8, u)
            if u < NH - 1:
                prep_qb(split_n(NH + u), u)

    r8q = lax.broadcasted_iota(jnp.int32, (8, TQ), 0)

    def group(j, carry, with_scores=True):
        h0 = NH * j
        n0 = i * H + h0
        ms = [m_ref[u] for u in range(NH)]
        acc = [None] * NH
        for u in range(NH):
            m8 = None
            if with_scores:
                hd = split_n(n0 + NH + u)
                if u == NH - 1:
                    prep_qb(hd, u)
            for c in range(NCK):
                acc[u] = softmax_pv(h0 + u, u, ms[u], c, acc[u])
                if with_scores:
                    m8 = scores(hd, u, c, m8, True)
                    if u > 0 and 1 <= c <= 3 * NT:
                        prep_part(split_n(n0 + 2 * NH + u - 1), u - 1,
                                  (c - 1) // NT, (c - 1) % NT, m8)
            if with_scores:
                finish_m(m8, u)
        for u in range(0, NH, 2):
            oe = acc[u] * (1.0 / acc[u][20:21])
            oo = acc[u + 1] * (1.0 / acc[u + 1][0:1])
            base = j * (DH * NH) + DH * u
            if not isinstance(base, int):
                base = pl.multiple_of(base, 8)
            ot_ref[pl.ds(base, 16), :] = oe[:16]
            ot_ref[pl.ds(base + 16, 8), :] = jnp.where(r8q < 4, oe[16:24], oo[:8])
            ot_ref[pl.ds(base + 24, 16), :] = oo[8:24]
        return carry

    lax.fori_loop(0, jnp.where(i == NQ - 1, NGRP - 1, NGRP), group, 0)

    @pl.when(i == NQ - 1)
    def _():
        group(NGRP - 1, 0, with_scores=False)

    @pl.when(i == 0)
    def _():
        for cp in late_copies:
            cp.wait()

    @pl.when(i > 0)
    def _():
        for t in range(ESPLIT):
            out_copy(i - 1, t).wait()

    hs = []
    for t in range(ESPLIT):
        o = ot_ref[:, pl.ds(t * R, R)].T.astype(BF16)
        r0 = pl.multiple_of(i * TQ + t * R, R)
        hs.append(x_ref[pl.ds(r0, R), :].astype(F32) + jnp.dot(
            o, wo_ref[...], preferred_element_type=F32))
    acts = []
    for t in range(ESPLIT):
        hn = _ln(hs[t]).astype(BF16)
        a = (jnp.dot(hn, w1_ref[...], preferred_element_type=F32)
             + b1_ref[...].astype(F32)[None, :])
        acts.append(_gelu(a).astype(BF16))
    for t in range(ESPLIT):
        y = (jnp.dot(acts[t], w2_ref[...], preferred_element_type=F32)
             + b2_ref[...].astype(F32)[None, :])
        o_ref[pl.ds(t * R, R), :] = (hs[t] + y).astype(BF16)
        out_copy(i, t).start()

    @pl.when(i == NQ - 1)
    def _():
        for t in range(ESPLIT):
            out_copy(i, t).wait()


@jax.jit
def pallas_sequential_preLN__softmax_full_mha__dense_activation_gelu__prompt_kernel(
    A_x: jax.Array,
    A_wqkv: jax.Array,
    A_wo: jax.Array,
    B_x: jax.Array,
    B_w1: jax.Array,
    B_b1: jax.Array,
    B_w2: jax.Array,
    B_b2: jax.Array,
):
    hbm = pl.BlockSpec(memory_space=pl.ANY)
    out = pl.pallas_call(
        _kernel,
        grid=(NQ,),
        in_specs=[hbm] * 7,
        out_specs=hbm,
        out_shape=jax.ShapeDtypeStruct((S, D), BF16),
        scratch_shapes=[
            pltpu.VMEM((S, D), BF16),
            pltpu.VMEM((D, D), BF16),
            pltpu.VMEM((2, D, D), BF16),
            pltpu.VMEM((D, D), BF16),
            pltpu.VMEM((D, F), BF16),
            pltpu.VMEM((F, D), BF16),
            pltpu.VMEM((S, D), BF16),
            pltpu.VMEM((2 * D, D), BF16),
            pltpu.VMEM((NPAIR, S // 2, 128), U32),
            pltpu.VMEM((NPAIR, NQ, 40, TQ), U32),
            pltpu.VMEM((H, 24, S), F32),
            pltpu.VMEM((NH, S, TQ), F32),
            pltpu.VMEM((NH, 8, TQ), F32),
            pltpu.VMEM((D, TQ), F32),
            pltpu.VMEM((NPAIR, NV, 128), U32),
            pltpu.VMEM((H, DH, NV, 128), F32),
            pltpu.VMEM((NPAIR, NQ, 40, TQ), F32),
            pltpu.VMEM((NH, DH, 8, TQ), F32),
            pltpu.VMEM((24, TQ), F32),
            pltpu.VMEM((4, KM // 2, D), U32),
            pltpu.VMEM((TQ, D), BF16),
            pltpu.VMEM((F,), BF16),
            pltpu.VMEM((D,), BF16),
            pltpu.SemaphoreType.DMA((len(XCH),)),
            pltpu.SemaphoreType.DMA((8,)),
            pltpu.SemaphoreType.DMA((ESPLIT,)),
        ],
        compiler_params=pltpu.CompilerParams(
            dimension_semantics=("arbitrary",),
            vmem_limit_bytes=124 * 1024 * 1024),
    )(A_x.reshape(S, D), A_wqkv, A_wo, B_w1, B_b1, B_w2, B_b2)
    return out.reshape(1, S, D)
```

```python
import math

import jax
import jax.numpy as jnp
from jax import lax
import jax.experimental.pallas as pl
import jax.experimental.pallas.tpu as pltpu

S = 2048
D = 640
H = 32
DH = 20
F = 1536
EPS = 1e-5
NG = D // 128
NPAIR = H // 2
LOG2E = 1.4426950408889634

F32 = jnp.float32
BF16 = jnp.bfloat16
U32 = jnp.uint32

TQ = 512
CK = 128
NQ = S // TQ
NCK = S // CK
NT = TQ // 128
NH = 4
NGRP = H // NH
ESPLIT = 4
R = TQ // ESPLIT
QSPLIT = 16
KM = 128
LM = 128
HPI = H // NQ
XCH = ((0, 256), (256, 512), (512, 1024), (1024, 2048))
KB4 = 1152
LSPLIT = 1536
LLEAD = 384
OFF = [0, 1, 2, 4, 5, 7, 8, 10, 11, 13]
NV = 16 * len(OFF)
NPC = 2 * len(OFF)
NSUB = 4
PPOS = [max(OFF[p // 2] * NSUB + NSUB - 1, 3 + (p * (NCK * NSUB - 3)) // NPC)
        for p in range(NPC)]


def _ln(x):
    m = jnp.mean(x, axis=-1, keepdims=True)
    xc = x - m
    v = jnp.mean(xc * xc, axis=-1, keepdims=True)
    return xc * lax.rsqrt(v + EPS)


def _gelu(x):
    c = math.sqrt(2.0 / math.pi)
    inner = x * (c + (c * 0.044715) * (x * x))
    return x * (0.5 + 0.5 * jnp.tanh(inner))


def _kernel(x_hbm, wqkv_hbm, wo_hbm, w1_hbm, b1_hbm, w2_hbm, b2_hbm, o_hbm,
            x_ref, wk_ref, wqv_ref, wo_ref, w1_ref, w2_ref,
            xn_ref, wt_ref, kp_ref, qh_ref, vt_ref, s_ref, m_ref, ot_ref,
            kw_ref, kb_ref, qth_ref, qb_ref, zero_ref, kraw_ref, o_ref, b1_ref, b2_ref,
            xsem, wsem, osem):
    i = pl.program_id(0)

    def x_copy(r):
        a, b = XCH[r]
        return pltpu.make_async_copy(
            x_hbm.at[pl.ds(a, b - a), :], x_ref.at[pl.ds(a, b - a), :], xsem.at[r])

    wk_copy = pltpu.make_async_copy(wqkv_hbm.at[:, pl.ds(D, D)], wk_ref, wsem.at[0])
    wq_copy = pltpu.make_async_copy(wqkv_hbm.at[:, pl.ds(0, D)], wqv_ref.at[0], wsem.at[1])
    wv_copy = pltpu.make_async_copy(wqkv_hbm.at[:, pl.ds(2 * D, D)], wqv_ref.at[1], wsem.at[2])
    late_copies = [
        pltpu.make_async_copy(wo_hbm, wo_ref, wsem.at[3]),
        pltpu.make_async_copy(w1_hbm, w1_ref, wsem.at[4]),
        pltpu.make_async_copy(w2_hbm, w2_ref, wsem.at[5]),
        pltpu.make_async_copy(b1_hbm, b1_ref, wsem.at[6]),
        pltpu.make_async_copy(b2_hbm, b2_ref, wsem.at[7]),
    ]

    def out_copy(step, t):
        r0 = pl.multiple_of(step * TQ + t * R, R)
        return pltpu.make_async_copy(
            o_ref.at[pl.ds(t * R, R), :], o_hbm.at[pl.ds(r0, R), :], osem.at[t])

    def split_n(n):
        if isinstance(n, int):
            return n % H, (n % H) // 2, min(n // H, NQ - 1)
        h = n & (H - 1)
        return h, h >> 1, jnp.minimum(n >> 5, NQ - 1)

    def prep_qb(hd, u):
        _, pr, qb = hd
        e = u % 2
        for a in range(2 * e, 2 * e + 3):
            q8 = qth_ref[pr, qb, pl.ds(8 * a, 8), :]
            for r in range(8):
                d = 8 * a + r - DH * e
                if 0 <= d < DH:
                    qb_ref[u, d] = jnp.broadcast_to(q8[r:r + 1], (8, TQ))

    def prep_part(hd, u, a, t, anchor):
        _, pr, qb = hd
        e = u % 2
        a = a + 2 * e
        q8 = qth_ref[pr, qb, pl.ds(8 * a, 8), pl.ds(t * 128, 128)]
        an = anchor[:, t * 128:(t + 1) * 128]
        q8 = jnp.where(an != an, an, q8)
        for r in range(8):
            d = 8 * a + r - DH * e
            if 0 <= d < DH:
                qb_ref[u, d, :, pl.ds(t * 128, 128)] = jnp.broadcast_to(q8[r:r + 1], (8, 128))

    def scores_vpu(hd, u, p, m8):
        kb = kb_ref[hd[0], :, pl.ds(p * 8, 8), :]
        kt = jnp.concatenate([kb] * NT, axis=2)
        q = qb_ref[u]
        sv = None
        for jd in range(DH // 2):
            for d in (jd, jd + DH // 2):
                a = kt[d] * q[d]
                sv = a if sv is None else sv + a
        s_ref[u, pl.ds(OFF[p // 2] * CK + (p % 2) * 8, 8), :] = sv
        return jnp.maximum(m8, sv)

    def scores(hd, u, c, m8, offload):
        _, pr, qb = hd
        e = u % 2
        kd = 48 if e else 32
        r0 = c * CK + (16 if (offload and c in OFF) else 0)
        nr = (c + 1) * CK - r0
        k = pltpu.bitcast(kp_ref[pr, pl.ds(r0 // 2, nr // 2), :], BF16)
        q = pltpu.bitcast(qh_ref[pr, qb, pl.ds(16 * e, kd // 2), :], BF16)
        s = jnp.dot(k[:, :kd], q, preferred_element_type=F32)
        s_ref[u, pl.ds(r0, nr), :] = s
        nsub = NSUB if offload else 1
        ng = nr // 8
        for qd in range(nsub):
            a, b = (qd * ng) // nsub, ((qd + 1) * ng) // nsub
            pm = jnp.max(s[a * 8:b * 8].reshape(b - a, 8, TQ), axis=0)
            m8 = pm if m8 is None else jnp.maximum(m8, pm)
            if offload:
                for p in range(NPC):
                    if PPOS[p] == c * NSUB + qd:
                        m8 = scores_vpu(hd, u, p, m8)
        return m8

    def finish_m(m8, u):
        m = jnp.max(m8, axis=0, keepdims=True)
        m_ref[u] = jnp.broadcast_to(m, (8, TQ))

    def softmax(u, m, c):
        s = s_ref[u, pl.ds(c * CK, CK), :].reshape(CK // 8, 8, TQ)
        return jnp.exp2(s - m[None]).reshape(CK, TQ)

    def pv(h, u, p, c, acc):
        o = jnp.dot(vt_ref[h, :, pl.ds(c * CK, CK)], p, preferred_element_type=F32)
        if acc is None:
            return (zero_ref[...] + o) if u > 0 else o
        return acc + o

    def ln_rows(a, b):
        for r0 in range(a, b, LM):
            xn_ref[pl.ds(r0, LM), :] = _ln(
                x_ref[pl.ds(r0, LM), :].astype(F32)).astype(BF16)

    def store_pairs(ku, r0):
        lane = lax.broadcasted_iota(jnp.int32, (KM // 2, 128), 1)
        for j in range(NPAIR):
            start = 2 * DH * j
            g0, g1 = start // 128, (start + 2 * DH - 1) // 128
            kk = ku[:, g0 * 128:(g0 + 1) * 128]
            if g1 != g0:
                kk = jnp.where(lane >= 64, kk, ku[:, g1 * 128:(g1 + 1) * 128])
            sh = (128 - start % 128) % 128
            if sh:
                kk = pltpu.roll(kk, sh, 1)
            kp_ref[j, pl.ds(r0 // 2, KM // 2), :] = kk

    def kproj_rows(a, b, defer_last=None):
        for r0 in range(a, b, KM):
            k = jnp.dot(xn_ref[pl.ds(r0, KM), :], wk_ref[...],
                        preferred_element_type=F32)
            ku = pltpu.bitcast(k.astype(BF16), U32)
            if defer_last is not None and r0 + KM == b:
                kraw_ref[defer_last] = ku
            else:
                store_pairs(ku, r0)

    def ln_and_kproj(lr, kr, slot):
        if slot > 0:
            store_pairs(kraw_ref[slot - 1], kr[0] - KM)
        ls = list(range(lr[0], lr[1], LM))
        ks = list(range(kr[0], kr[1], KM))
        for n, k0 in enumerate(ks):
            for l0 in ls[(n * len(ls)) // len(ks):((n + 1) * len(ls)) // len(ks)]:
                ln_rows(l0, l0 + LM)
            kproj_rows(k0, k0 + KM, slot if k0 + KM == kr[1] else None)

    def build_kw():
        for j in range(NPAIR):
            ku = jnp.concatenate(
                [kp_ref[j, pl.ds(c * CK // 2, 8), :] for c in OFF], axis=0)
            kk = pltpu.bitcast(ku, BF16).astype(F32)
            kb = pltpu.bitcast(kk, U32)
            kw_ref[j] = ((pltpu.roll(kb, 128 - DH // 2, 1) & jnp.uint32(0xFFFF0000))
                         | (kb >> 16))

    def build_kb(pr, e):
        kw = kw_ref[pr]
        for jd in range(DH // 2):
            l = DH * e + jd
            w = jnp.broadcast_to(kw[:, l:l + 1], (NV, 128))
            kb_ref[2 * pr + e, jd] = pltpu.bitcast(w << 16, F32)
            kb_ref[2 * pr + e, jd + DH // 2] = pltpu.bitcast(
                w & jnp.uint32(0xFFFF0000), F32)

    @pl.when(i == 0)
    def _prologue():
        x_copy(0).start()
        wk_copy.start()
        zero_ref[...] = jnp.zeros((24, TQ), F32)
        x_copy(1).start()
        x_copy(0).wait()
        x_copy(2).start()
        ln_rows(*XCH[0])
        wk_copy.wait()
        x_copy(1).wait()
        x_copy(3).start()
        ln_and_kproj(XCH[1], XCH[0], 0)
        x_copy(2).wait()
        wq_copy.start()
        wv_copy.start()
        ln_and_kproj(XCH[2], XCH[1], 1)
        x_copy(3).wait()
        ln_and_kproj((XCH[3][0], LSPLIT), (XCH[2][0], KB4), 2)
        wq_copy.wait()
        wv_copy.wait()
        for cp in late_copies:
            cp.start()
        store_pairs(kraw_ref[2], KB4 - KM)
        for t in range(2):
            for b in range(NG):
                wt_ref[pl.ds(t * D + b * 128, 128), :] = (
                    wqv_ref[t, :, pl.ds(b * 128, 128)].astype(F32).T.astype(BF16))
        for k0 in range(KB4, (OFF[-1] + 1) * CK, KM):
            if LSPLIT <= k0 + LLEAD < S:
                ln_rows(k0 + LLEAD, k0 + LLEAD + KM)
            kproj_rows(k0, k0 + KM)
        build_kw()
        kproj_rows((OFF[-1] + 1) * CK, S, 3)

        qscale = (DH ** -0.5) * LOG2E
        r24 = lax.broadcasted_iota(jnp.int32, (24, TQ), 0)
        r32 = lax.broadcasted_iota(jnp.int32, (32, TQ), 0)

        def qv_step(r, carry):
            r0 = pl.multiple_of(r * TQ, TQ)
            xn = xn_ref[pl.ds(r0, TQ), :]
            zero16 = jnp.zeros((8, TQ), U32)
            mr = 2 * D // QSPLIT
            pps = mr // (2 * DH)
            for b in range(QSPLIT):
                for hh in range((b * HPI) // QSPLIT, ((b + 1) * HPI) // QSPLIT):
                    build_kb(r * (HPI // 2) + hh // 2, hh % 2)
                qv = lax.dot_general(wt_ref[pl.ds(b * mr, mr), :], xn,
                                     (((1,), (1,)), ((), ())),
                                     preferred_element_type=F32)
                for jj in range(pps):
                    g = b * pps + jj
                    blk = qv[40 * jj:40 * jj + 40]
                    if g < NPAIR:
                        q = blk * qscale
                        qe = jnp.where(r32 < DH, q[:32], 0.0).astype(BF16)
                        qo = jnp.concatenate(
                            [jnp.where(r24 >= 4, q[16:40], 0.0),
                             jnp.zeros((8, TQ), F32)], axis=0).astype(BF16)
                        qh_ref[g, r, pl.ds(0, 16), :] = pltpu.bitcast(qe, U32)
                        qh_ref[g, r, pl.ds(16, 8), :] = zero16
                        qh_ref[g, r, pl.ds(24, 16), :] = pltpu.bitcast(qo, U32)
                        qth_ref[g, r] = q.astype(BF16).astype(F32)
                    else:
                        j = g - NPAIR
                        ve = jnp.where(r24 < DH, blk[:24], jnp.where(r24 == DH, 1.0, 0.0))
                        vt_ref[2 * j, :, pl.ds(r0, TQ)] = ve.astype(BF16).astype(F32)
                        vo = jnp.where(r24 >= 4, blk[16:40], jnp.where(r24 == 0, 1.0, 0.0))
                        vt_ref[2 * j + 1, :, pl.ds(r0, TQ)] = vo.astype(BF16).astype(F32)
            return carry

        lax.fori_loop(0, NQ, qv_step, 0)

        store_pairs(kraw_ref[3], S - KM)
        for u in range(NH):
            m8 = None
            for c in range(NCK):
                m8 = scores(split_n(u), u, c, m8, False)
            finish_m(m8, u)
            for v in {NH - 2: (u, u + 1), NH - 1: ()}.get(u, (u,)):
                prep_qb(split_n(NH + v), v)

    r8q = lax.broadcasted_iota(jnp.int32, (8, TQ), 0)

    def group(j, carry, with_scores=True):
        h0 = NH * j
        n0 = i * H + h0
        ms = [m_ref[u] for u in range(NH)]
        acc = [None] * NH
        for u in range(NH):
            m8 = None
            if with_scores:
                hd = split_n(n0 + NH + u)
            for c in range(NCK):
                p = softmax(u, ms[u], c)
                if with_scores:
                    m8 = scores(hd, u, c, m8, True)
                acc[u] = pv(h0 + u, u, p, c, acc[u])
                if with_scores and u > 0 and 1 <= c <= 3 * NT:
                    prep_part(split_n(n0 + 2 * NH + u - 1), u - 1,
                              (c - 1) // NT, (c - 1) % NT, m8)
            if with_scores:
                finish_m(m8, u)
                if u == NH - 1:
                    prep_qb(split_n(n0 + 2 * NH + u), u)
        for u in range(0, NH, 2):
            oe = acc[u] * (1.0 / acc[u][20:21])
            oo = acc[u + 1] * (1.0 / acc[u + 1][0:1])
            base = j * (DH * NH) + DH * u
            if not isinstance(base, int):
                base = pl.multiple_of(base, 8)
            ot_ref[pl.ds(base, 16), :] = oe[:16]
            ot_ref[pl.ds(base + 16, 8), :] = jnp.where(r8q < 4, oe[16:24], oo[:8])
            ot_ref[pl.ds(base + 24, 16), :] = oo[8:24]
        return carry

    lax.fori_loop(0, jnp.where(i == NQ - 1, NGRP - 1, NGRP), group, 0)

    @pl.when(i == NQ - 1)
    def _():
        group(NGRP - 1, 0, with_scores=False)

    @pl.when(i == 0)
    def _():
        for cp in late_copies:
            cp.wait()

    @pl.when(i > 0)
    def _():
        for t in range(ESPLIT):
            out_copy(i - 1, t).wait()

    hs = []
    for t in range(ESPLIT):
        o = ot_ref[:, pl.ds(t * R, R)].T.astype(BF16)
        r0 = pl.multiple_of(i * TQ + t * R, R)
        hs.append(x_ref[pl.ds(r0, R), :].astype(F32) + jnp.dot(
            o, wo_ref[...], preferred_element_type=F32))
    acts = []
    for t in range(ESPLIT):
        hn = _ln(hs[t]).astype(BF16)
        a = (jnp.dot(hn, w1_ref[...], preferred_element_type=F32)
             + b1_ref[...].astype(F32)[None, :])
        acts.append(_gelu(a).astype(BF16))
    for t in range(ESPLIT):
        y = (jnp.dot(acts[t], w2_ref[...], preferred_element_type=F32)
             + b2_ref[...].astype(F32)[None, :])
        o_ref[pl.ds(t * R, R), :] = (hs[t] + y).astype(BF16)
        out_copy(i, t).start()

    @pl.when(i == NQ - 1)
    def _():
        for t in range(ESPLIT):
            out_copy(i, t).wait()


@jax.jit
def pallas_sequential_preLN__softmax_full_mha__dense_activation_gelu__prompt_kernel(
    A_x: jax.Array,
    A_wqkv: jax.Array,
    A_wo: jax.Array,
    B_x: jax.Array,
    B_w1: jax.Array,
    B_b1: jax.Array,
    B_w2: jax.Array,
    B_b2: jax.Array,
):
    hbm = pl.BlockSpec(memory_space=pl.ANY)
    out = pl.pallas_call(
        _kernel,
        grid=(NQ,),
        in_specs=[hbm] * 7,
        out_specs=hbm,
        out_shape=jax.ShapeDtypeStruct((S, D), BF16),
        scratch_shapes=[
            pltpu.VMEM((S, D), BF16),
            pltpu.VMEM((D, D), BF16),
            pltpu.VMEM((2, D, D), BF16),
            pltpu.VMEM((D, D), BF16),
            pltpu.VMEM((D, F), BF16),
            pltpu.VMEM((F, D), BF16),
            pltpu.VMEM((S, D), BF16),
            pltpu.VMEM((2 * D, D), BF16),
            pltpu.VMEM((NPAIR, S // 2, 128), U32),
            pltpu.VMEM((NPAIR, NQ, 40, TQ), U32),
            pltpu.VMEM((H, 24, S), F32),
            pltpu.VMEM((NH, S, TQ), F32),
            pltpu.VMEM((NH, 8, TQ), F32),
            pltpu.VMEM((D, TQ), F32),
            pltpu.VMEM((NPAIR, NV, 128), U32),
            pltpu.VMEM((H, DH, NV, 128), F32),
            pltpu.VMEM((NPAIR, NQ, 40, TQ), F32),
            pltpu.VMEM((NH, DH, 8, TQ), F32),
            pltpu.VMEM((24, TQ), F32),
            pltpu.VMEM((4, KM // 2, D), U32),
            pltpu.VMEM((TQ, D), BF16),
            pltpu.VMEM((F,), BF16),
            pltpu.VMEM((D,), BF16),
            pltpu.SemaphoreType.DMA((len(XCH),)),
            pltpu.SemaphoreType.DMA((8,)),
            pltpu.SemaphoreType.DMA((ESPLIT,)),
        ],
        compiler_params=pltpu.CompilerParams(
            dimension_semantics=("arbitrary",),
            vmem_limit_bytes=124 * 1024 * 1024),
    )(A_x.reshape(S, D), A_wqkv, A_wo, B_w1, B_b1, B_w2, B_b2)
    return out.reshape(1, S, D)
```

```python
import math

import jax
import jax.numpy as jnp
from jax import lax
import jax.experimental.pallas as pl
import jax.experimental.pallas.tpu as pltpu

S = 2048
D = 640
H = 32
DH = 20
F = 1536
EPS = 1e-5
NG = D // 128
NPAIR = H // 2
LOG2E = 1.4426950408889634

F32 = jnp.float32
BF16 = jnp.bfloat16
U32 = jnp.uint32

TQ = 512
CK = 128
NQ = S // TQ
NCK = S // CK
NT = TQ // 128
NH = 4
NGRP = H // NH
ESPLIT = 4
R = TQ // ESPLIT
QSPLIT = 16
KM = 128
LM = 128
HPI = H // NQ
XCH = ((0, 256), (256, 512), (512, 1024), (1024, 2048))
KB4 = 1152
LSPLIT = 1536
LLEAD = 384
OFF = [0, 1, 2, 4, 5, 7, 8, 10, 11, 13]
NV = 16 * len(OFF)
NPC = 2 * len(OFF)
NSUB = 4
PPOS = [max(OFF[p // 2] * NSUB + NSUB - 1, 3 + (p * (NCK * NSUB - 3)) // NPC)
        for p in range(NPC)]


def _ln(x):
    m = jnp.mean(x, axis=-1, keepdims=True)
    xc = x - m
    v = jnp.mean(xc * xc, axis=-1, keepdims=True)
    return xc * lax.rsqrt(v + EPS)


def _gelu(x):
    c = math.sqrt(2.0 / math.pi)
    inner = x * (c + (c * 0.044715) * (x * x))
    return x * (0.5 + 0.5 * jnp.tanh(inner))


def _kernel(x_hbm, wqkv_hbm, wo_hbm, w1_hbm, b1_hbm, w2_hbm, b2_hbm, o_hbm,
            x_ref, wk_ref, wqv_ref, wo_ref, w1_ref, w2_ref,
            xn_ref, wt_ref, kp_ref, qh_ref, vt_ref, s_ref, m_ref, ot_ref,
            kw_ref, kb_ref, qth_ref, qb_ref, zero_ref, kraw_ref, o_ref, b1_ref, b2_ref,
            xsem, wsem, osem):
    i = pl.program_id(0)

    def x_copy(r):
        a, b = XCH[r]
        return pltpu.make_async_copy(
            x_hbm.at[pl.ds(a, b - a), :], x_ref.at[pl.ds(a, b - a), :], xsem.at[r])

    wk_copy = pltpu.make_async_copy(wqkv_hbm.at[:, pl.ds(D, D)], wk_ref, wsem.at[0])
    wq_copy = pltpu.make_async_copy(wqkv_hbm.at[:, pl.ds(0, D)], wqv_ref.at[0], wsem.at[1])
    wv_copy = pltpu.make_async_copy(wqkv_hbm.at[:, pl.ds(2 * D, D)], wqv_ref.at[1], wsem.at[2])
    late_copies = [
        pltpu.make_async_copy(wo_hbm, wo_ref, wsem.at[3]),
        pltpu.make_async_copy(w1_hbm, w1_ref, wsem.at[4]),
        pltpu.make_async_copy(w2_hbm, w2_ref, wsem.at[5]),
        pltpu.make_async_copy(b1_hbm, b1_ref, wsem.at[6]),
        pltpu.make_async_copy(b2_hbm, b2_ref, wsem.at[7]),
    ]

    def out_copy(step, t):
        r0 = pl.multiple_of(step * TQ + t * R, R)
        return pltpu.make_async_copy(
            o_ref.at[pl.ds(t * R, R), :], o_hbm.at[pl.ds(r0, R), :], osem.at[t])

    def split_n(n):
        if isinstance(n, int):
            return n % H, (n % H) // 2, min(n // H, NQ - 1)
        h = n & (H - 1)
        return h, h >> 1, jnp.minimum(n >> 5, NQ - 1)

    def prep_part(hd, u, a, lanes, anchor=None):
        _, pr, qb = hd
        e = u % 2
        a = a + 2 * e
        l0, nl = lanes
        q8 = qth_ref[pr, qb, pl.ds(8 * a, 8), pl.ds(l0, nl)]
        if anchor is not None:
            an = anchor[:, l0:l0 + nl]
            q8 = jnp.where(an != an, an, q8)
        rows = [r for r in range(8) if 0 <= 8 * a + r - DH * e < DH]
        qb_ref[u, pl.ds(8 * a + rows[0] - DH * e, len(rows)), :, pl.ds(l0, nl)] = jnp.stack(
            [jnp.broadcast_to(q8[r:r + 1], (8, nl)) for r in rows])

    def prep_qb(hd, u):
        for a in range(3):
            prep_part(hd, u, a, (0, TQ))

    def scores_vpu(hd, u, p, m8):
        kb = kb_ref[hd[0], :, pl.ds(p * 8, 8), :]
        kt = jnp.concatenate([kb] * NT, axis=2)
        q = qb_ref[u]
        sv = None
        for jd in range(DH // 2):
            for d in (jd, jd + DH // 2):
                a = kt[d] * q[d]
                sv = a if sv is None else sv + a
        s_ref[u, pl.ds(OFF[p // 2] * CK + (p % 2) * 8, 8), :] = sv
        return jnp.maximum(m8, sv)

    def scores(hd, u, c, m8, offload):
        _, pr, qb = hd
        e = u % 2
        kd = 48 if e else 32
        r0 = c * CK + (16 if (offload and c in OFF) else 0)
        nr = (c + 1) * CK - r0
        k = pltpu.bitcast(kp_ref[pr, pl.ds(r0 // 2, nr // 2), :], BF16)
        q = pltpu.bitcast(qh_ref[pr, qb, pl.ds(16 * e, kd // 2), :], BF16)
        s = jnp.dot(k[:, :kd], q, preferred_element_type=F32)
        s_ref[u, pl.ds(r0, nr), :] = s
        nsub = NSUB if offload else 1
        ng = nr // 8
        for qd in range(nsub):
            a, b = (qd * ng) // nsub, ((qd + 1) * ng) // nsub
            pm = jnp.max(s[a * 8:b * 8].reshape(b - a, 8, TQ), axis=0)
            m8 = pm if m8 is None else jnp.maximum(m8, pm)
            if offload:
                for p in range(NPC):
                    if PPOS[p] == c * NSUB + qd:
                        m8 = scores_vpu(hd, u, p, m8)
        return m8

    def finish_m(m8, u):
        m = jnp.max(m8, axis=0, keepdims=True)
        m_ref[u] = jnp.broadcast_to(m, (8, TQ))

    def softmax(u, m, c):
        s = s_ref[u, pl.ds(c * CK, CK), :].reshape(CK // 8, 8, TQ)
        return jnp.exp2(s - m[None]).reshape(CK, TQ)

    def pv(h, u, p, c, acc):
        o = jnp.dot(vt_ref[h, :, pl.ds(c * CK, CK)], p, preferred_element_type=F32)
        if acc is None:
            return (zero_ref[...] + o) if u > 0 else o
        return acc + o

    def ln_rows(a, b):
        for r0 in range(a, b, LM):
            xn_ref[pl.ds(r0, LM), :] = _ln(
                x_ref[pl.ds(r0, LM), :].astype(F32)).astype(BF16)

    def store_pairs(ku, r0):
        lane = lax.broadcasted_iota(jnp.int32, (KM // 2, 128), 1)
        for j in range(NPAIR):
            start = 2 * DH * j
            g0, g1 = start // 128, (start + 2 * DH - 1) // 128
            kk = ku[:, g0 * 128:(g0 + 1) * 128]
            if g1 != g0:
                kk = jnp.where(lane >= 64, kk, ku[:, g1 * 128:(g1 + 1) * 128])
            sh = (128 - start % 128) % 128
            if sh:
                kk = pltpu.roll(kk, sh, 1)
            kp_ref[j, pl.ds(r0 // 2, KM // 2), :] = kk

    def kproj_rows(a, b, defer_last=None):
        for r0 in range(a, b, KM):
            k = jnp.dot(xn_ref[pl.ds(r0, KM), :], wk_ref[...],
                        preferred_element_type=F32)
            ku = pltpu.bitcast(k.astype(BF16), U32)
            if defer_last is not None and r0 + KM == b:
                kraw_ref[defer_last] = ku
            else:
                store_pairs(ku, r0)

    def ln_and_kproj(lr, kr, slot):
        if slot > 0:
            store_pairs(kraw_ref[slot - 1], kr[0] - KM)
        ls = list(range(lr[0], lr[1], LM))
        ks = list(range(kr[0], kr[1], KM))
        for n, k0 in enumerate(ks):
            for l0 in ls[(n * len(ls)) // len(ks):((n + 1) * len(ls)) // len(ks)]:
                ln_rows(l0, l0 + LM)
            kproj_rows(k0, k0 + KM, slot if k0 + KM == kr[1] else None)

    def build_kw():
        for j in range(NPAIR):
            ku = jnp.concatenate(
                [kp_ref[j, pl.ds(c * CK // 2, 8), :] for c in OFF], axis=0)
            kk = pltpu.bitcast(ku, BF16).astype(F32)
            kb = pltpu.bitcast(kk, U32)
            kw_ref[j] = ((pltpu.roll(kb, 128 - DH // 2, 1) & jnp.uint32(0xFFFF0000))
                         | (kb >> 16))

    def build_kb(pr, e):
        kw = kw_ref[pr]
        for jd in range(DH // 2):
            l = DH * e + jd
            w = jnp.broadcast_to(kw[:, l:l + 1], (NV, 128))
            kb_ref[2 * pr + e, jd] = pltpu.bitcast(w << 16, F32)
            kb_ref[2 * pr + e, jd + DH // 2] = pltpu.bitcast(
                w & jnp.uint32(0xFFFF0000), F32)

    @pl.when(i == 0)
    def _prologue():
        x_copy(0).start()
        wk_copy.start()
        zero_ref[...] = jnp.zeros((24, TQ), F32)
        x_copy(1).start()
        x_copy(0).wait()
        x_copy(2).start()
        ln_rows(*XCH[0])
        wk_copy.wait()
        x_copy(1).wait()
        x_copy(3).start()
        ln_and_kproj(XCH[1], XCH[0], 0)
        x_copy(2).wait()
        wq_copy.start()
        wv_copy.start()
        ln_and_kproj(XCH[2], XCH[1], 1)
        x_copy(3).wait()
        ln_and_kproj((XCH[3][0], LSPLIT), (XCH[2][0], KB4), 2)
        wq_copy.wait()
        wv_copy.wait()
        for cp in late_copies:
            cp.start()
        store_pairs(kraw_ref[2], KB4 - KM)
        for t in range(2):
            for b in range(NG):
                wt_ref[pl.ds(t * D + b * 128, 128), :] = (
                    wqv_ref[t, :, pl.ds(b * 128, 128)].astype(F32).T.astype(BF16))
        for k0 in range(KB4, (OFF[-1] + 1) * CK, KM):
            if LSPLIT <= k0 + LLEAD < S:
                ln_rows(k0 + LLEAD, k0 + LLEAD + KM)
            kproj_rows(k0, k0 + KM)
        build_kw()
        kproj_rows((OFF[-1] + 1) * CK, S, 3)

        qscale = (DH ** -0.5) * LOG2E
        r24 = lax.broadcasted_iota(jnp.int32, (24, TQ), 0)
        r32 = lax.broadcasted_iota(jnp.int32, (32, TQ), 0)

        def qv_step(r, carry):
            r0 = pl.multiple_of(r * TQ, TQ)
            xn = xn_ref[pl.ds(r0, TQ), :]
            zero16 = jnp.zeros((8, TQ), U32)
            mr = 2 * D // QSPLIT
            pps = mr // (2 * DH)
            for b in range(QSPLIT):
                for hh in range((b * HPI) // QSPLIT, ((b + 1) * HPI) // QSPLIT):
                    build_kb(r * (HPI // 2) + hh // 2, hh % 2)
                qv = lax.dot_general(wt_ref[pl.ds(b * mr, mr), :], xn,
                                     (((1,), (1,)), ((), ())),
                                     preferred_element_type=F32)
                for jj in range(pps):
                    g = b * pps + jj
                    blk = qv[40 * jj:40 * jj + 40]
                    if g < NPAIR:
                        q = blk * qscale
                        qe = jnp.where(r32 < DH, q[:32], 0.0).astype(BF16)
                        qo = jnp.concatenate(
                            [jnp.where(r24 >= 4, q[16:40], 0.0),
                             jnp.zeros((8, TQ), F32)], axis=0).astype(BF16)
                        qh_ref[g, r, pl.ds(0, 16), :] = pltpu.bitcast(qe, U32)
                        qh_ref[g, r, pl.ds(16, 8), :] = zero16
                        qh_ref[g, r, pl.ds(24, 16), :] = pltpu.bitcast(qo, U32)
                        qth_ref[g, r] = q.astype(BF16).astype(F32)
                    else:
                        j = g - NPAIR
                        ve = jnp.where(r24 < DH, blk[:24], jnp.where(r24 == DH, 1.0, 0.0))
                        vt_ref[2 * j, :, pl.ds(r0, TQ)] = ve.astype(BF16).astype(F32)
                        vo = jnp.where(r24 >= 4, blk[16:40], jnp.where(r24 == 0, 1.0, 0.0))
                        vt_ref[2 * j + 1, :, pl.ds(r0, TQ)] = vo.astype(BF16).astype(F32)
            return carry

        lax.fori_loop(0, NQ, qv_step, 0)

        store_pairs(kraw_ref[3], S - KM)
        for u in range(NH):
            m8 = None
            for c in range(NCK):
                m8 = scores(split_n(u), u, c, m8, False)
            finish_m(m8, u)
            for v in {NH - 2: (u, u + 1), NH - 1: ()}.get(u, (u,)):
                prep_qb(split_n(NH + v), v)

    r8q = lax.broadcasted_iota(jnp.int32, (8, TQ), 0)

    def group(j, carry, with_scores=True):
        h0 = NH * j
        n0 = i * H + h0
        ms = [m_ref[u] for u in range(NH)]
        acc = [None] * NH
        for u in range(NH):
            m8 = None
            if with_scores:
                hd = split_n(n0 + NH + u)
            for c in range(NCK):
                p = softmax(u, ms[u], c)
                if with_scores:
                    m8 = scores(hd, u, c, m8, True)
                acc[u] = pv(h0 + u, u, p, c, acc[u])
                if with_scores and u > 0 and 1 <= c <= 3 * NT:
                    prep_part(split_n(n0 + 2 * NH + u - 1), u - 1,
                              (c - 1) // NT, (((c - 1) % NT) * 128, 128), m8)
            if with_scores:
                finish_m(m8, u)
                if u == NH - 1:
                    prep_qb(split_n(n0 + 2 * NH + u), u)
        for u in range(0, NH, 2):
            oe = acc[u] * (1.0 / acc[u][20:21])
            oo = acc[u + 1] * (1.0 / acc[u + 1][0:1])
            base = j * (DH * NH) + DH * u
            if not isinstance(base, int):
                base = pl.multiple_of(base, 8)
            ot_ref[pl.ds(base, 16), :] = oe[:16]
            ot_ref[pl.ds(base + 16, 8), :] = jnp.where(r8q < 4, oe[16:24], oo[:8])
            ot_ref[pl.ds(base + 24, 16), :] = oo[8:24]
        return carry

    lax.fori_loop(0, jnp.where(i == NQ - 1, NGRP - 1, NGRP), group, 0)

    @pl.when(i == NQ - 1)
    def _():
        group(NGRP - 1, 0, with_scores=False)

    @pl.when(i == 0)
    def _():
        for cp in late_copies:
            cp.wait()

    @pl.when(i > 0)
    def _():
        for t in range(ESPLIT):
            out_copy(i - 1, t).wait()

    hs = []
    for t in range(ESPLIT):
        o = ot_ref[:, pl.ds(t * R, R)].T.astype(BF16)
        r0 = pl.multiple_of(i * TQ + t * R, R)
        hs.append(x_ref[pl.ds(r0, R), :].astype(F32) + jnp.dot(
            o, wo_ref[...], preferred_element_type=F32))
    acts = []
    for t in range(ESPLIT):
        hn = _ln(hs[t]).astype(BF16)
        a = (jnp.dot(hn, w1_ref[...], preferred_element_type=F32)
             + b1_ref[...].astype(F32)[None, :])
        acts.append(_gelu(a).astype(BF16))
    for t in range(ESPLIT):
        y = (jnp.dot(acts[t], w2_ref[...], preferred_element_type=F32)
             + b2_ref[...].astype(F32)[None, :])
        o_ref[pl.ds(t * R, R), :] = (hs[t] + y).astype(BF16)
        out_copy(i, t).start()

    @pl.when(i == NQ - 1)
    def _():
        for t in range(ESPLIT):
            out_copy(i, t).wait()


@jax.jit
def pallas_sequential_preLN__softmax_full_mha__dense_activation_gelu__prompt_kernel(
    A_x: jax.Array,
    A_wqkv: jax.Array,
    A_wo: jax.Array,
    B_x: jax.Array,
    B_w1: jax.Array,
    B_b1: jax.Array,
    B_w2: jax.Array,
    B_b2: jax.Array,
):
    hbm = pl.BlockSpec(memory_space=pl.ANY)
    out = pl.pallas_call(
        _kernel,
        grid=(NQ,),
        in_specs=[hbm] * 7,
        out_specs=hbm,
        out_shape=jax.ShapeDtypeStruct((S, D), BF16),
        scratch_shapes=[
            pltpu.VMEM((S, D), BF16),
            pltpu.VMEM((D, D), BF16),
            pltpu.VMEM((2, D, D), BF16),
            pltpu.VMEM((D, D), BF16),
            pltpu.VMEM((D, F), BF16),
            pltpu.VMEM((F, D), BF16),
            pltpu.VMEM((S, D), BF16),
            pltpu.VMEM((2 * D, D), BF16),
            pltpu.VMEM((NPAIR, S // 2, 128), U32),
            pltpu.VMEM((NPAIR, NQ, 40, TQ), U32),
            pltpu.VMEM((H, 24, S), F32),
            pltpu.VMEM((NH, S, TQ), F32),
            pltpu.VMEM((NH, 8, TQ), F32),
            pltpu.VMEM((D, TQ), F32),
            pltpu.VMEM((NPAIR, NV, 128), U32),
            pltpu.VMEM((H, DH, NV, 128), F32),
            pltpu.VMEM((NPAIR, NQ, 40, TQ), F32),
            pltpu.VMEM((NH, DH, 8, TQ), F32),
            pltpu.VMEM((24, TQ), F32),
            pltpu.VMEM((4, KM // 2, D), U32),
            pltpu.VMEM((TQ, D), BF16),
            pltpu.VMEM((F,), BF16),
            pltpu.VMEM((D,), BF16),
            pltpu.SemaphoreType.DMA((len(XCH),)),
            pltpu.SemaphoreType.DMA((8,)),
            pltpu.SemaphoreType.DMA((ESPLIT,)),
        ],
        compiler_params=pltpu.CompilerParams(
            dimension_semantics=("arbitrary",),
            vmem_limit_bytes=124 * 1024 * 1024),
    )(A_x.reshape(S, D), A_wqkv, A_wo, B_w1, B_b1, B_w2, B_b2)
    return out.reshape(1, S, D)
```
